```python
import jax
import jax.numpy as jnp

def _softmax(x, axis=-1):
    return jax.nn.softmax(x, axis=axis)

def _gelu(x):
    return jax.nn.gelu(x, approximate=True)

def _silu(x):
    return jax.nn.silu(x)

def _sigmoid(x):
    return jax.nn.sigmoid(x)

def _layernorm(x, axis=-1, eps=1e-05):
    m = jnp.mean(x, axis=axis, keepdims=True)
    v = jnp.var(x, axis=axis, keepdims=True)
    return (x - m) / jnp.sqrt(v + eps)

def _scatter_add(tgt, idx, src, axis=0):
    return tgt.at[idx].add(src)

def _segment_sum(src, seg, n):
    return jax.ops.segment_sum(src, seg, n)

class _Rng:

    def __init__(self, key):
        self._k = key

    def _next(self):
        self._k, sub = jax.random.split(self._k)
        return sub

    def normal(self, shape):
        return jax.random.normal(self._next(), shape, dtype=jnp.bfloat16)

    def randint(self, lo, hi, shape):
        return jax.random.randint(self._next(), shape, lo, hi, dtype=jnp.int32)

    def uniform(self, shape, lo=0.0, hi=1.0):
        return jax.random.uniform(self._next(), shape, jnp.bfloat16, lo, hi)

    def permutation(self, n):
        return jax.random.permutation(self._next(), n)
kernel_name = 'adaLN_cond__memory_aug_recurrent_mem_tr__mixer_s_mlp__prompt'

def setup_inputs():
    _rng = _Rng(jax.random.key(int.from_bytes(__import__("os").urandom(4), "little")))
    _w = lambda a: (lambda t: t.astype(jnp.bfloat16) if jnp.issubdtype(t.dtype, jnp.floating) else t)(jnp.asarray(a))

    def _A_setup():
        B, S, Dm = (1, 2048, 1024)
        H, Dh = (32, 128)
        M, seg = (8, 32)
        seg = min(seg, S)
        S = S // seg * seg
        return {'x': _w((lambda *s: _rng.normal(s) * 0.05)(B, S, Dm)), 'mem0': _w((lambda *s: _rng.normal(s) * 0.05)(B, M, Dm)), 'Wq': _w((lambda *s: _rng.normal(s) * 0.05)(Dm, H, Dh) * Dm ** (-0.5)), 'Wk': _w((lambda *s: _rng.normal(s) * 0.05)(Dm, H, Dh) * Dm ** (-0.5)), 'Wv': _w((lambda *s: _rng.normal(s) * 0.05)(Dm, H, Dh) * Dm ** (-0.5)), 'Wo': _w((lambda *s: _rng.normal(s) * 0.05)(H, Dh, Dm) * (H * Dh) ** (-0.5)), 'seg_len': seg}
    _A_in = _A_setup()

    def _B_setup():
        B, S, D, F = (1, 2048, 1024, 3584)
        return {'x': _w((lambda *s: _rng.normal(s) * 0.05)(B, S, D)), 'w1': _w((lambda *s: _rng.normal(s) * 0.05)(D, D) * D ** (-0.5)), 'w2': _w((lambda *s: _rng.normal(s) * 0.05)(D, D) * D ** (-0.5)), 'w3': _w((lambda *s: _rng.normal(s) * 0.05)(D, F) * D ** (-0.5)), 'w4': _w((lambda *s: _rng.normal(s) * 0.05)(F, D) * F ** (-0.5))}
    _B_in = _B_setup()
    return {'A_x': _A_in['x'], 'A_mem0': _A_in['mem0'], 'A_Wq': _A_in['Wq'], 'A_Wk': _A_in['Wk'], 'A_Wv': _A_in['Wv'], 'A_Wo': _A_in['Wo'], 'A_seg_len': _A_in['seg_len'], 'B_x': _B_in['x'], 'B_w1': _B_in['w1'], 'B_w2': _B_in['w2'], 'B_w3': _B_in['w3'], 'B_w4': _B_in['w4'], 'c': _w((lambda *s: _rng.normal(s) * 0.05)(1, 1024)), 'w_mod': _w((lambda *s: _rng.normal(s) * 0.05)(1024, 6 * 1024) * 1024 ** (-0.5))}

def reference(A_x, A_mem0, A_Wq, A_Wk, A_Wv, A_Wo, A_seg_len, B_x, B_w1, B_w2, B_w3, B_w4, c, w_mod):

    def _A_ref(x, mem0, Wq, Wk, Wv, Wo, seg_len):
        B, S, Dm = x.shape
        H, Dh = (Wq.shape[1], Wq.shape[2])
        M = mem0.shape[1]
        scale = Dh ** (-0.5)
        n_seg = S // seg_len
        L = M + seg_len
        idx = jnp.arange(L)
        mask = (idx[:, None] < M) | (idx[:, None] >= idx[None, :])
        mem = mem0
        outs = []
        for s in range(n_seg):
            xs = x[:, s * seg_len:(s + 1) * seg_len, :].copy()
            h = jnp.concatenate([mem, xs], axis=1)
            q = jnp.einsum('btd,dhe->bhte', h, Wq)
            k = jnp.einsum('btd,dhe->bhte', h, Wk)
            v = jnp.einsum('btd,dhe->bhte', h, Wv)
            scores = jnp.einsum('bhqe,bhke->bhqk', q, k) * scale
            scores = jnp.where(mask[None, None], scores, -1000000000.0)
            p = _softmax(scores, axis=-1)
            o = jnp.einsum('bhqk,bhke->bhqe', p, v)
            o = jnp.einsum('bhte,hed->btd', o, Wo)
            mem = o[:, :M, :].copy()
            outs.append(o[:, M:, :])
        return jnp.concatenate(outs, axis=1)

    def _B_ref(x, w1, w2, w3, w4):
        B, S, D = x.shape
        h = _gelu(_layernorm(x, axis=-1) @ w1)
        c = D // 4
        g0 = jnp.pad(h[:, :, 0 * c:1 * c], ((0, 0), (1, 0), (0, 0)))[:, :S, :]
        g1 = jnp.pad(h[:, :, 1 * c:2 * c], ((0, 0), (0, 1), (0, 0)))[:, 1:, :]
        g2 = jnp.pad(h[:, :, 2 * c:3 * c], ((0, 0), (2, 0), (0, 0)))[:, :S, :]
        g3 = jnp.pad(h[:, :, 3 * c:], ((0, 0), (0, 2), (0, 0)))[:, 2:, :]
        hs = jnp.concatenate([g0, g1, g2, g3], axis=-1) @ w2
        x1 = x + hs
        h2 = _gelu(_layernorm(x1, axis=-1) @ w3) @ w4
        return x1 + h2
    x = A_x
    mod = (_silu(c) @ w_mod).reshape(c.shape[0], 6, 1, -1)
    sa, ca, ga, sb, cb, gb = (mod[:, 0].copy(), mod[:, 1].copy(), mod[:, 2].copy(), mod[:, 3].copy(), mod[:, 4].copy(), mod[:, 5].copy())
    h = _layernorm(x, axis=-1) * (1 + ca) + sa
    x = x + ga * _A_ref(h, A_mem0, A_Wq, A_Wk, A_Wv, A_Wo, A_seg_len)
    h = _layernorm(x, axis=-1) * (1 + cb) + sb
    x = x + gb * _B_ref(h, B_w1, B_w2, B_w3, B_w4)
    return x
```

```python
import functools

import jax
import jax.numpy as jnp
import numpy as np
import jax.experimental.pallas as pl
import jax.experimental.pallas.tpu as pltpu

F32 = jnp.float32
BF16 = jnp.bfloat16
U32 = jnp.uint32
LANES = 128
EPS = 1e-5
LOG2E = 1.4426950408889634


def _ln(x):
    m = jnp.mean(x, axis=-1, keepdims=True)
    d = x - m
    v = jnp.mean(d * d, axis=-1, keepdims=True)
    return d * jax.lax.rsqrt(v + EPS)


def _gelu(x):
    c0 = float(np.sqrt(2.0 / np.pi))
    inner = x * (c0 + (c0 * 0.044715) * (x * x))
    hx = 0.5 * x
    return hx + hx * jnp.tanh(inner)


def _dot(a, b):
    return jnp.dot(a, b, preferred_element_type=F32)


def _dot_nt(a, b):
    return jax.lax.dot_general(a, b, (((1,), (1,)), ((), ())),
                               preferred_element_type=F32)


def _attn_fill(n_mem, n_loop, n_pre):
    head = np.concatenate([np.zeros(n_loop), np.ones(n_loop),
                           np.zeros(n_pre), np.ones(n_pre)])
    tok = np.concatenate([np.arange(n_loop), np.arange(n_loop),
                          n_loop + np.arange(n_pre), n_loop + np.arange(n_pre)])
    same = head[:, None] == head[None, :]
    vis = (tok[:, None] < n_mem) | (tok[:, None] >= tok[None, :])
    fill = np.where(same, np.where(vis, 0.0, -1e9 * LOG2E), -np.inf)
    return fill.astype(np.float32)


def _kernel(x_hbm, mem0_ref, wq_hbm, wk_hbm, wv_hbm, wo_hbm, w1_hbm, w2_hbm, w3_hbm,
            w4_hbm, c_ref, wmod_hbm, fill_ref, out_hbm,
            x_v, buf, wqkv, wo_v, pre, odef, mod_v, sems,
            *, S, D, H, DH, M, SEG, FF, TB, FC):
    NSEG = S // SEG
    NL = 32
    NX = NL - M
    NP = SEG - NX
    HP = H // 2
    NCT = D // LANES
    scale = float(DH) ** -0.5 * LOG2E

    def wtile(j):
        return pltpu.bitcast(wqkv[j], BF16)

    def prologue(wmod_v, stage, hpre):
        cp_m0 = pltpu.make_async_copy(wmod_hbm.at[:, pl.ds(0, 2 * D)],
                                      wmod_v.at[:, pl.ds(0, 2 * D)], sems.at[0])
        cp_m1 = pltpu.make_async_copy(wmod_hbm.at[:, pl.ds(2 * D, 4 * D)],
                                      wmod_v.at[:, pl.ds(2 * D, 4 * D)], sems.at[1])
        cp_x = pltpu.make_async_copy(x_hbm, x_v, sems.at[2])
        cp_w = [pltpu.make_async_copy(w.bitcast(U32), stage.at[i], sems.at[3 + i])
                for i, w in enumerate((wq_hbm, wk_hbm, wv_hbm))]
        cp_o = [pltpu.make_async_copy(wo_hbm.at[:, pl.ds(j * LANES, LANES)],
                                      wo_v.at[j], sems.at[6 + j]) for j in range(NCT)]
        cp_m0.start()
        cp_x.start()
        cp_w[0].start()

        cv = c_ref[...].astype(F32)
        sc = jnp.broadcast_to(cv * jax.nn.sigmoid(cv), (16, D)).astype(BF16)
        cp_m0.wait()
        mod_v[:, 0:2 * D] = _dot(sc, wmod_v[:, 0:2 * D])[0:8]
        cp_x.wait()
        cp_w[1].start()

        sa = mod_v[0:1, 0:D]
        ca1 = 1.0 + mod_v[0:1, D:2 * D]

        def ln_body(i, _):
            r = pl.ds(pl.multiple_of(i * (2 * SEG), 2 * SEG), 2 * SEG)
            h = _ln(x_v[r, :].astype(F32)) * ca1 + sa
            buf[r, :] = h
            hp_ = jnp.concatenate([h[NX:SEG], h[SEG + NX:2 * SEG]], axis=0)
            hpre[pl.ds(pl.multiple_of(i * (2 * NP), 2 * NP), 2 * NP), :] = hp_.astype(BF16)
            return 0

        jax.lax.fori_loop(0, NSEG // 2, ln_body, 0)

        st32 = stage
        for mat in range(3):
            cp_w[mat].wait()
            if mat == 0:
                cp_w[2].start()
            elif mat == 1:
                for cp in cp_o:
                    cp.start()
            else:
                cp_m1.start()

            def hp_body(hp, _, mat=mat):
                we = st32[mat, pl.ds(hp, D // 2, stride=H), :]
                wo_ = st32[mat, pl.ds(hp + HP, D // 2, stride=H), :]
                w0 = (we & 0xFFFF) | (wo_ << 16)
                w1 = (we >> 16) | (wo_ & np.uint32(0xFFFF0000))
                j = mat * H + 2 * hp
                wqkv[j] = w0
                wqkv[j + 1] = w1
                lhs = hpre[...]
                a = _dot(lhs, pltpu.bitcast(w0, BF16)).reshape(NSEG, NP, DH)
                b = _dot(lhs, pltpu.bitcast(w1, BF16)).reshape(NSEG, NP, DH)
                pre[mat * HP + hp] = jnp.concatenate([a, b], axis=1).astype(BF16)
                return 0

            jax.lax.fori_loop(0, HP, hp_body, 0)

        for cp in cp_o:
            cp.wait()
        cp_m1.wait()
        mod_v[:, 2 * D:6 * D] = _dot(sc, wmod_v[:, 2 * D:6 * D])[0:8]

    pl.run_scoped(prologue,
                  pltpu.VMEM((D, 6 * D), BF16),
                  pltpu.VMEM((3, D * H // 2, DH), U32),
                  pltpu.VMEM((NSEG * NP, D), BF16))

    def main(w1_v, w2_v, w3_v, w4_v, ubuf, hbuf, obuf, osem):
        cps = [pltpu.make_async_copy(s_, d_, sems.at[i]) for i, (s_, d_) in enumerate(
            ((w1_hbm, w1_v), (w2_hbm, w2_v), (w3_hbm, w3_v), (w4_hbm, w4_v)))]
        for cp in cps:
            cp.start()

        def seg_body(s, mem):
            r0 = pl.multiple_of(s * SEG, SEG)
            lhs = jnp.concatenate([mem, buf[pl.ds(r0, NX), :]], axis=0).astype(BF16)
            fill = fill_ref[...]
            vis = fill == 0.0

            def proj(mat, hp):
                a = _dot(lhs, wtile(mat * H + 2 * hp))
                b = _dot(lhs, wtile(mat * H + 2 * hp + 1))
                ab = jnp.concatenate([a, b], axis=0).astype(BF16)
                return jnp.concatenate([ab, pre[mat * HP + hp, s]], axis=0)

            def probs(q, k):
                sc_ = jnp.where(vis, _dot_nt(q, k) * scale, fill)
                e = jnp.exp2(sc_ - jnp.max(sc_, axis=-1, keepdims=True))
                return e.astype(BF16), 1.0 / jnp.sum(e, axis=-1, keepdims=True)

            outs = []

            def finish(hp, e, inv, v):
                o = (_dot(e, v) * inv).astype(BF16)
                outs.append(o[0:NL])
                outs.append(o[NL:2 * NL])
                odef[hp, s] = o[2 * NL:]

            q, k, v, pr = {}, {}, {}, {}
            for hp in range(HP + 2):
                if hp < HP:
                    q[hp] = proj(0, hp)
                    k[hp] = proj(1, hp)
                if 0 <= hp - 1 < HP:
                    pr[hp - 1] = probs(q[hp - 1], k[hp - 1])
                if 0 <= hp - 1 < HP:
                    v[hp - 1] = proj(2, hp - 1)
                if 0 <= hp - 2 < HP:
                    finish(hp - 2, *pr[hp - 2], v[hp - 2])
            half = H // 2
            o_lo = jnp.concatenate(outs[:half], axis=1)
            o_hi = jnp.concatenate(outs[half:], axis=1)
            acc = [_dot(o_lo, wo_v[j, 0:half * DH, :]) for j in range(NCT)]
            res = jnp.concatenate(
                [acc[j] + _dot(o_hi, wo_v[j, half * DH:H * DH, :]) for j in range(NCT)], axis=1)
            buf[pl.ds(r0, NX), :] = res[M:]
            return res[:M]

        jax.lax.fori_loop(0, NSEG, seg_body, mem0_ref[...].astype(F32))

        for cp in cps:
            cp.wait()

        ga = mod_v[0:1, 2 * D:3 * D]
        sb = mod_v[0:1, 3 * D:4 * D]
        cb1 = 1.0 + mod_v[0:1, 4 * D:5 * D]
        gb = mod_v[0:1, 5 * D:6 * D]
        NS = TB // SEG
        PAD = 8
        ubuf[:, 0:PAD, :] = jnp.zeros((NCT, PAD, LANES), F32)
        ubuf[:, PAD + S:2 * PAD + S, :] = jnp.zeros((NCT, PAD, LANES), F32)

        def stage1(c, _):
            r = pl.ds(pl.multiple_of(c * TB, TB), TB)
            s0 = pl.ds(c * NS, NS)
            cols = []
            for hp in range(HP):
                od = odef[hp, s0].astype(F32)
                cols.append(od[:, 0:NP].reshape(NS * NP, DH).astype(BF16))
                cols.append(od[:, NP:2 * NP].reshape(NS * NP, DH).astype(BF16))
            od = jnp.concatenate(cols, axis=1)
            ad = jnp.concatenate([_dot(od, wo_v[j]) for j in range(NCT)], axis=1)
            al = buf[r, :].reshape(NS, SEG, D)[:, 0:NX]
            att = jnp.concatenate([al, ad.reshape(NS, NP, D)], axis=1).reshape(TB, D)
            x1 = x_v[r, :].astype(F32) + ga * att
            buf[r, :] = x1
            h = _ln(x1) * cb1 + sb
            hbuf[r, :] = h
            u = _gelu(_dot(_ln(h).astype(BF16), w1_v[...]))
            ru = pl.ds(pl.multiple_of(c * TB + PAD, 8), TB)
            for j in range(NCT):
                ubuf[j, ru, :] = u[:, j * LANES:(j + 1) * LANES]
            return 0

        jax.lax.fori_loop(0, S // TB, stage1, 0)

        def out_copy(c):
            r = pl.ds(pl.multiple_of(c * TB, TB), TB)
            return pltpu.make_async_copy(obuf.at[r], out_hbm.at[r], osem.at[c])

        shifts = (-1, 1, -2, 2)

        def stage2(c, _):
            r = pl.ds(pl.multiple_of(c * TB, TB), TB)
            g = jnp.concatenate(
                [ubuf[j, pl.ds(c * TB + PAD + shifts[j * 4 // NCT], TB), :]
                 for j in range(NCT)], axis=1).astype(BF16)
            y = hbuf[r, :] + _dot(g, w2_v[...])
            yn = _ln(y).astype(BF16)
            acc = y
            for f in range(FF // FC):
                t = _gelu(_dot(yn, w3_v[:, f * FC:(f + 1) * FC])).astype(BF16)
                acc = acc + _dot(t, w4_v[f * FC:(f + 1) * FC, :])
            obuf[r, :] = (buf[r, :] + gb * acc).astype(BF16)
            out_copy(c).start()
            return 0

        jax.lax.fori_loop(0, S // TB, stage2, 0)
        for c in range(S // TB):
            out_copy(c).wait()

    pl.run_scoped(main,
                  pltpu.VMEM((D, D), BF16),
                  pltpu.VMEM((D, D), BF16),
                  pltpu.VMEM((D, FF), BF16),
                  pltpu.VMEM((FF, D), BF16),
                  pltpu.VMEM((NCT, S + 16, LANES), F32),
                  pltpu.VMEM((S, D), F32),
                  pltpu.VMEM((S, D), BF16),
                  pltpu.SemaphoreType.DMA((S // TB,)))


@functools.partial(jax.jit, static_argnames=("A_seg_len",))
def pallas_adaLN_cond__memory_aug_recurrent_mem_tr__mixer_s_mlp__prompt_kernel(
    A_x, A_mem0, A_Wq, A_Wk, A_Wv, A_Wo, A_seg_len, B_x, B_w1, B_w2, B_w3, B_w4, c, w_mod,
):
    del B_x
    B, S, D = A_x.shape
    _, H, DH = A_Wq.shape
    M = A_mem0.shape[1]
    SEG = int(A_seg_len)
    FF = B_w3.shape[1]
    assert B == 1 and DH == LANES and M == 8 and SEG == 32 and S % SEG == 0
    NSEG = S // SEG
    NP = SEG - (32 - M)
    fill = _attn_fill(M, 32, NP)

    hbm = pl.BlockSpec(memory_space=pl.ANY)
    vmem = pl.BlockSpec(memory_space=pltpu.VMEM)
    out = pl.pallas_call(
        functools.partial(_kernel, S=S, D=D, H=H, DH=DH, M=M, SEG=SEG, FF=FF, TB=256, FC=512),
        out_shape=jax.ShapeDtypeStruct((S, D), A_x.dtype),
        in_specs=[hbm, vmem, hbm, hbm, hbm, hbm, hbm, hbm, hbm, hbm, vmem, hbm, vmem],
        out_specs=hbm,
        scratch_shapes=[
            pltpu.VMEM((S, D), BF16),
            pltpu.VMEM((S, D), F32),
            pltpu.VMEM((3 * H, D // 2, DH), U32),
            pltpu.VMEM((D // LANES, H * DH, LANES), BF16),
            pltpu.VMEM((3 * H // 2, NSEG, 2 * NP, DH), BF16),
            pltpu.VMEM((H // 2, NSEG, 2 * NP, DH), BF16),
            pltpu.VMEM((8, 6 * D), F32),
            pltpu.SemaphoreType.DMA((6 + D // LANES,)),
        ],
        compiler_params=pltpu.CompilerParams(vmem_limit_bytes=126 * 2**20),
        name="adaln_rmt_mixer",
    )(
        A_x.reshape(S, D), A_mem0.reshape(M, D),
        A_Wq.reshape(D * H, DH), A_Wk.reshape(D * H, DH), A_Wv.reshape(D * H, DH),
        A_Wo.reshape(H * DH, D), B_w1, B_w2, B_w3, B_w4, c, w_mod, fill,
    )
    return out.reshape(B, S, D)
```

```python
import functools

import jax
import jax.numpy as jnp
import numpy as np
import jax.experimental.pallas as pl
import jax.experimental.pallas.tpu as pltpu

F32 = jnp.float32
BF16 = jnp.bfloat16
U32 = jnp.uint32
LANES = 128
EPS = 1e-5
LOG2E = 1.4426950408889634
NL = 32


def _ln(x):
    m = jnp.mean(x, axis=-1, keepdims=True)
    d = x - m
    v = jnp.mean(d * d, axis=-1, keepdims=True)
    return d * jax.lax.rsqrt(v + EPS)


def _gelu(x):
    c0 = float(np.sqrt(2.0 / np.pi))
    inner = x * (c0 + (c0 * 0.044715) * (x * x))
    hx = 0.5 * x
    return hx + hx * jnp.tanh(inner)


def _dot(a, b):
    return jnp.dot(a, b, preferred_element_type=F32)


def _dot_nt(a, b):
    return jax.lax.dot_general(a, b, (((1,), (1,)), ((), ())),
                               preferred_element_type=F32)


def _bf(words):
    return pltpu.bitcast(words, BF16)


def _words(x):
    return pltpu.bitcast(x.astype(BF16), U32)


def _attn_fill(n_mem, n_loop, n_pre):
    head = np.concatenate([np.zeros(n_loop), np.ones(n_loop),
                           np.zeros(n_pre), np.ones(n_pre)])
    tok = np.concatenate([np.arange(n_loop), np.arange(n_loop),
                          n_loop + np.arange(n_pre), n_loop + np.arange(n_pre)])
    same = head[:, None] == head[None, :]
    vis = (tok[:, None] < n_mem) | (tok[:, None] >= tok[None, :])
    fill = np.where(same, np.where(vis, 0.0, -1e9 * LOG2E), -np.inf)
    return fill.astype(np.float32)


def _kernel(x_hbm, mem0_ref, wq_hbm, wk_hbm, wv_hbm, wo_hbm, w1_hbm, w2_hbm, w3_hbm,
            w4_hbm, c_ref, wmod_hbm, fill_ref, out_hbm,
            x_v, xpre, hpre, hnext, buf, wqkv, wo_v, pre, odef, mod_v, wmod_v,
            w1_v, w2_v, w3_v, w4_v, ubuf, hbuf, obuf, wsem, sems, osem,
            *, S, D, H, DH, M, SEG, FF, TA, TB, FC, SU):
    NSEG = S // SEG
    NX = NL - M
    NP = SEG - NX
    HP = H // 2
    NCT = D // LANES
    scale = float(DH) ** -0.5 * LOG2E

    x32 = x_hbm.bitcast(U32)
    wmod32 = wmod_hbm.bitcast(U32)
    cp_xpre = pltpu.make_async_copy(x32.at[:, pl.ds(NX // 2, NP // 2), :], xpre, sems.at[0])
    cp_m0 = pltpu.make_async_copy(wmod32.at[:, pl.ds(0, 2 * D)],
                                  wmod_v.at[:, pl.ds(0, 2 * D)], sems.at[1])
    cp_m1 = pltpu.make_async_copy(wmod32.at[:, pl.ds(2 * D, 4 * D)],
                                  wmod_v.at[:, pl.ds(2 * D, 4 * D)], sems.at[2])
    cp_x = pltpu.make_async_copy(x32, x_v, sems.at[3])
    cp_o = pltpu.make_async_copy(wo_hbm.bitcast(U32), wo_v, sems.at[4])
    cp_b = [pltpu.make_async_copy(s_.bitcast(U32), d_, sems.at[5 + i])
            for i, (s_, d_) in enumerate(
                ((w1_hbm, w1_v), (w2_hbm, w2_v), (w3_hbm, w3_v), (w4_hbm, w4_v)))]

    cp_xpre.start()
    cp_m0.start()

    def fetch_pair(hp):
        for mat, w in enumerate((wq_hbm, wk_hbm, wv_hbm)):
            for par in range(2):
                pltpu.make_async_copy(w.bitcast(U32).at[:, par, hp, :],
                                      wqkv.at[6 * hp + 2 * mat + par], wsem.at[hp]).start()

    AHEAD = HP // 2
    for hp in range(AHEAD):
        fetch_pair(hp)

    cv = c_ref[...].astype(F32)
    silu_c = jnp.broadcast_to(cv * jax.nn.sigmoid(cv), (16, D)).astype(BF16)
    with jax.named_scope('P_wait_xpre'):
        cp_xpre.wait()
    xn = _ln(_bf(xpre[...]).astype(F32).reshape(NSEG * NP, D))
    buf[0:NSEG * NP, :] = xn
    with jax.named_scope('P_wait_m0'):
        cp_m0.wait()
    mod_v[:, 0:2 * D] = _dot(silu_c, _bf(wmod_v[:, 0:2 * D]))[0:8]
    sa = mod_v[0:1, 0:D]
    ca1 = 1.0 + mod_v[0:1, D:2 * D]
    hpre[...] = _words(buf[0:NSEG * NP, :] * ca1 + sa)

    def pre_body(hp, _):
        @pl.when(hp + AHEAD < HP)
        def _():
            fetch_pair(hp + AHEAD)

        @pl.when(hp + AHEAD == HP)
        def _():
            for cp in [cp_x, cp_o, cp_m1] + cp_b:
                cp.start()

        slabs = wqkv.at[pl.ds(6 * hp, 6)]
        pltpu.make_async_copy(slabs, slabs, wsem.at[hp]).wait()
        for mat in range(3):
            we = wqkv[6 * hp + 2 * mat]
            wo_ = wqkv[6 * hp + 2 * mat + 1]
            w0 = (we & 0xFFFF) | (wo_ << 16)
            w1 = (we >> 16) | (wo_ & np.uint32(0xFFFF0000))
            wqkv[6 * hp + 2 * mat] = w0
            wqkv[6 * hp + 2 * mat + 1] = w1
            lhs = _bf(hpre[...])
            a = _dot(lhs, _bf(w0)).reshape(NSEG, NP, DH)
            b = _dot(lhs, _bf(w1)).reshape(NSEG, NP, DH)
            pre[3 * hp + mat] = _words(
                jnp.concatenate([a, b], axis=1).reshape(NSEG * 2 * NP, DH))
        return 0

    with jax.named_scope("P_pre"):
        jax.lax.fori_loop(0, HP, pre_body, 0)

    def modulated(s):
        return _ln(_bf(x_v[s]).astype(F32)[0:NX]) * ca1 + sa

    cp_x.wait()
    hnext[...] = modulated(0)
    cp_o.wait()

    def seg_step(s, mem):
        lhs = jnp.concatenate([mem, hnext[...]], axis=0).astype(BF16)
        hnext[...] = modulated(jnp.minimum(s + 1, NSEG - 1))
        rp = pl.ds(pl.multiple_of(s * NP, NP), NP)
        fill = fill_ref[...]
        vis = fill == 0.0

        def join(mat, hp, a, b):
            ab = jnp.concatenate([a, b], axis=0).astype(BF16)
            return jnp.concatenate([ab, _bf(pre[3 * hp + mat, rp, :])], axis=0)

        def proj(mat, hp):
            j = 6 * hp + 2 * mat
            return join(mat, hp, _dot(lhs, _bf(wqkv[j])), _dot(lhs, _bf(wqkv[j + 1])))

        def probs(q, k):
            sc = jnp.where(vis, _dot_nt(q, k) * scale, fill)
            e = jnp.exp2(sc - jnp.max(sc, axis=-1, keepdims=True))
            den = jnp.sum(e, axis=-1, keepdims=True)
            inv = pl.reciprocal(den, approx=True)
            inv = inv * (2.0 - den * inv)
            return (e * inv).astype(BF16)

        outs = []

        def finish(hp, p, v):
            o = _words(_dot(p, v))
            outs.append(o[0:NL // 2])
            outs.append(o[NL // 2:NL])
            odef[hp, rp, :] = o[NL:]

        def wo_part(h0, h1, j):
            return _dot(_bf(jnp.concatenate(outs[h0:h1], axis=1)),
                        _bf(wo_v[h0 * DH // 2:h1 * DH // 2, j * LANES:(j + 1) * LANES]))

        q, k, v, pr = {}, {}, {}, {}
        js = [2, 3, 0, 1]
        lo = [_dot(lhs[:, :D // 2], _bf(wqkv[j, 0:D // 4, :])) for j in js]
        full = [_dot(lhs[:, D // 2:], _bf(wqkv[j, D // 4:D // 2, :])) + a for a, j in zip(lo, js)]
        k[0] = join(1, 0, full[0], full[1])
        q[0] = join(0, 0, full[2], full[3])
        for hp in range(1, HP):
            k[hp] = proj(1, hp)
            pr[hp - 1] = probs(q[hp - 1], k[hp - 1])
            q[hp] = proj(0, hp)
            if hp >= 2:
                finish(hp - 2, pr[hp - 2], v[hp - 2])
            v[hp - 1] = proj(2, hp - 1)
        half = H // 2
        v[HP - 1] = proj(2, HP - 1)
        pr[HP - 1] = probs(q[HP - 1], k[HP - 1])
        acc = [wo_part(0, half, 0)]
        finish(HP - 2, pr[HP - 2], v[HP - 2])
        acc += [wo_part(0, half, j) for j in range(1, NCT // 2)]
        finish(HP - 1, pr[HP - 1], v[HP - 1])
        acc += [wo_part(0, half, j) for j in range(NCT // 2, NCT)]
        res = jnp.concatenate([wo_part(half, H, j) + acc[j] for j in range(NCT)], axis=1)
        buf[pl.ds(pl.multiple_of(s * SEG, SEG), NX), :] = res[M:]
        return res[:M]

    def seg_body(i, mem):
        for u in range(SU):
            mem = seg_step(i * SU + u, mem)
        return mem

    with jax.named_scope("P_seg"):
        jax.lax.fori_loop(0, NSEG // SU, seg_body, mem0_ref[...].astype(F32))

    cp_m1.wait()
    mod_v[:, 2 * D:6 * D] = _dot(silu_c, _bf(wmod_v[:, 2 * D:6 * D]))[0:8]
    for cp in cp_b:
        cp.wait()

    ga = mod_v[0:1, 2 * D:3 * D]
    sb = mod_v[0:1, 3 * D:4 * D]
    cb1 = 1.0 + mod_v[0:1, 4 * D:5 * D]
    gb = mod_v[0:1, 5 * D:6 * D]
    PAD = 8
    ubuf[:, 0:PAD, :] = jnp.zeros((NCT, PAD, LANES), F32)
    ubuf[:, PAD + S:2 * PAD + S, :] = jnp.zeros((NCT, PAD, LANES), F32)

    def stage1(c, _):
        th = TA // 2
        ns = th // SEG
        hn = []
        for t in range(2):
            r = pl.ds(pl.multiple_of(c * TA + t * th, th), th)
            s0 = pl.ds((2 * c + t) * ns, ns)
            rp = pl.ds(pl.multiple_of((2 * c + t) * (ns * NP), ns * NP), ns * NP)
            cols = []
            for hp in range(HP):
                od = _bf(odef[hp, rp, :]).astype(F32).reshape(ns, 2 * NP, DH)
                cols.append(od[:, 0:NP].reshape(ns * NP, DH))
                cols.append(od[:, NP:2 * NP].reshape(ns * NP, DH))
            ad = _dot(jnp.concatenate(cols, axis=1).astype(BF16), _bf(wo_v[...]))
            al = buf[r, :].reshape(ns, SEG, D)[:, 0:NX]
            att = jnp.concatenate([al, ad.reshape(ns, NP, D)], axis=1).reshape(th, D)
            x1 = _bf(x_v[s0].reshape(th // 2, D)).astype(F32) + ga * att
            buf[r, :] = x1
            h = _ln(x1) * cb1 + sb
            hbuf[r, :] = h
            hn.append(_ln(h).astype(BF16))
        for t in range(2):
            u = _gelu(_dot(hn[t], _bf(w1_v[...])))
            ru = pl.ds(pl.multiple_of(c * TA + t * th + PAD, 8), th)
            for j in range(NCT):
                ubuf[j, ru, :] = u[:, j * LANES:(j + 1) * LANES]
        return 0

    with jax.named_scope("P_s1"):
        jax.lax.fori_loop(0, S // TA, stage1, 0)

    out32 = out_hbm.bitcast(U32)

    def out_copy(c):
        r = pl.ds(pl.multiple_of(c * (TB // 2), TB // 2), TB // 2)
        return pltpu.make_async_copy(obuf.at[r], out32.at[r], osem.at[c])

    shifts = (-1, 1, -2, 2)

    def stage2(c, _):
        th = TB // 2
        ys = []
        for t in range(2):
            r0 = c * TB + t * th
            g = jnp.concatenate(
                [ubuf[j, pl.ds(r0 + PAD + shifts[j * 4 // NCT], th), :]
                 for j in range(NCT)], axis=1).astype(BF16)
            ys.append(_dot(g, _bf(w2_v[...])) + hbuf[pl.ds(pl.multiple_of(r0, th), th), :])
        yns = [_ln(y).astype(BF16) for y in ys]

        def up(yn, f):
            return _gelu(_dot(yn, _bf(w3_v[:, f * FC:(f + 1) * FC]))).astype(BF16)

        acc = jnp.concatenate(ys, axis=0)
        yn = jnp.concatenate(yns, axis=0)
        t_cur = jnp.concatenate([up(y, 0) for y in yns], axis=0)
        for f in range(FF // FC):
            t_next = up(yn, f + 1) if f + 1 < FF // FC else None
            acc = _dot(t_cur, _bf(w4_v[f * FC // 2:(f + 1) * FC // 2, :])) + acc
            t_cur = t_next
        r = pl.ds(pl.multiple_of(c * TB, TB), TB)
        obuf[pl.ds(pl.multiple_of(c * (TB // 2), TB // 2), TB // 2), :] = _words(
            buf[r, :] + gb * acc)
        out_copy(c).start()
        return 0

    with jax.named_scope("P_s2"):
        jax.lax.fori_loop(0, S // TB, stage2, 0)
    for c in range(S // TB):
        out_copy(c).wait()


@functools.partial(jax.jit, static_argnames=("A_seg_len",))
def pallas_adaLN_cond__memory_aug_recurrent_mem_tr__mixer_s_mlp__prompt_kernel(
    A_x, A_mem0, A_Wq, A_Wk, A_Wv, A_Wo, A_seg_len, B_x, B_w1, B_w2, B_w3, B_w4, c, w_mod,
):
    del B_x
    B, S, D = A_x.shape
    _, H, DH = A_Wq.shape
    M = A_mem0.shape[1]
    SEG = int(A_seg_len)
    FF = B_w3.shape[1]
    assert B == 1 and DH == LANES and M == 8 and SEG == 32 and S % SEG == 0
    NSEG = S // SEG
    NX = NL - M
    NP = SEG - NX
    TB = 256
    fill = _attn_fill(M, NL, NP)

    hbm = pl.BlockSpec(memory_space=pl.ANY)
    vmem = pl.BlockSpec(memory_space=pltpu.VMEM)
    out = pl.pallas_call(
        functools.partial(_kernel, S=S, D=D, H=H, DH=DH, M=M, SEG=SEG, FF=FF,
                          TA=512, TB=TB, FC=512, SU=2),
        out_shape=jax.ShapeDtypeStruct((S, D), A_x.dtype),
        in_specs=[hbm, vmem, hbm, hbm, hbm, hbm, hbm, hbm, hbm, hbm, vmem, hbm, vmem],
        out_specs=hbm,
        scratch_shapes=[
            pltpu.VMEM((NSEG, SEG // 2, D), U32),
            pltpu.VMEM((NSEG, NP // 2, D), U32),
            pltpu.VMEM((NSEG * NP // 2, D), U32),
            pltpu.VMEM((NX, D), F32),
            pltpu.VMEM((S, D), F32),
            pltpu.VMEM((3 * H, D // 2, DH), U32),
            pltpu.VMEM((H * DH // 2, D), U32),
            pltpu.VMEM((3 * H // 2, NSEG * NP, DH), U32),
            pltpu.VMEM((H // 2, NSEG * NP, DH), U32),
            pltpu.VMEM((8, 6 * D), F32),
            pltpu.VMEM((D // 2, 6 * D), U32),
            pltpu.VMEM((D // 2, D), U32),
            pltpu.VMEM((D // 2, D), U32),
            pltpu.VMEM((D // 2, FF), U32),
            pltpu.VMEM((FF // 2, D), U32),
            pltpu.VMEM((D // LANES, S + 16, LANES), F32),
            pltpu.VMEM((S, D), F32),
            pltpu.VMEM((S // 2, D), U32),
            pltpu.SemaphoreType.DMA((H // 2,)),
            pltpu.SemaphoreType.DMA((9,)),
            pltpu.SemaphoreType.DMA((S // TB,)),
        ],
        compiler_params=pltpu.CompilerParams(vmem_limit_bytes=127 * 2**20),
        name="adaln_rmt_mixer",
    )(
        A_x.reshape(NSEG, SEG, D), A_mem0.reshape(M, D),
        A_Wq.reshape(D // 2, 2, H, DH), A_Wk.reshape(D // 2, 2, H, DH),
        A_Wv.reshape(D // 2, 2, H, DH),
        A_Wo.reshape(H * DH, D), B_w1, B_w2, B_w3, B_w4, c, w_mod, fill,
    )
    return out.reshape(B, S, D)
```

```python
import functools

import jax
import jax.numpy as jnp
import numpy as np
import jax.experimental.pallas as pl
import jax.experimental.pallas.tpu as pltpu

F32 = jnp.float32
BF16 = jnp.bfloat16
U32 = jnp.uint32
LANES = 128
EPS = 1e-5
LOG2E = 1.4426950408889634
NL = 32


def _ln(x):
    m = jnp.mean(x, axis=-1, keepdims=True)
    d = x - m
    v = jnp.mean(d * d, axis=-1, keepdims=True)
    return d * jax.lax.rsqrt(v + EPS)


def _gelu(x):
    c0 = float(np.sqrt(2.0 / np.pi))
    inner = x * (c0 + (c0 * 0.044715) * (x * x))
    hx = 0.5 * x
    return hx + hx * jnp.tanh(inner)


def _dot(a, b):
    return jnp.dot(a, b, preferred_element_type=F32)


def _dot_nt(a, b):
    return jax.lax.dot_general(a, b, (((1,), (1,)), ((), ())),
                               preferred_element_type=F32)


def _bf(words):
    return pltpu.bitcast(words, BF16)


def _words(x):
    return pltpu.bitcast(x.astype(BF16), U32)


def _attn_fill(n_mem, n_loop, n_pre):
    head = np.concatenate([np.zeros(n_loop), np.ones(n_loop),
                           np.zeros(n_pre), np.ones(n_pre)])
    tok = np.concatenate([np.arange(n_loop), np.arange(n_loop),
                          n_loop + np.arange(n_pre), n_loop + np.arange(n_pre)])
    same = head[:, None] == head[None, :]
    vis = (tok[:, None] < n_mem) | (tok[:, None] >= tok[None, :])
    fill = np.where(same, np.where(vis, 0.0, -1e9 * LOG2E), -np.inf)
    return fill.astype(np.float32)


def _kernel(x_hbm, mem0_ref, wq_hbm, wk_hbm, wv_hbm, wo_hbm, w1_hbm, w2_hbm, w3_hbm,
            w4_hbm, c_ref, wmod_hbm, fill_ref, out_hbm,
            x_v, xpre, hpre, hnext, aprev, hnl, buf, wqkv, wo_v, pre, odef, mod_v, wmod_v,
            w1_v, w2_v, w3_v, w4_v, ubuf, hbuf, obuf, wsem, sems, osem,
            *, S, D, H, DH, M, SEG, FF, TA, TB, FC, SU):
    NSEG = S // SEG
    NX = NL - M
    NP = SEG - NX
    HP = H // 2
    NCT = D // LANES
    scale = float(DH) ** -0.5 * LOG2E

    x32 = x_hbm.bitcast(U32)
    wmod32 = wmod_hbm.bitcast(U32)
    cp_xpre = pltpu.make_async_copy(x32.at[:, pl.ds(NX // 2, NP // 2), :], xpre, sems.at[0])
    MC = D // 2
    cp_m0 = [pltpu.make_async_copy(wmod32.at[:, pl.ds(i * MC, MC)],
                                   wmod_v.at[:, pl.ds(i * MC, MC)], sems.at[9 + i])
             for i in range(2 * D // MC)]
    cp_m1 = pltpu.make_async_copy(wmod32.at[:, pl.ds(2 * D, 4 * D)],
                                  wmod_v.at[:, pl.ds(2 * D, 4 * D)], sems.at[2])
    cp_x = pltpu.make_async_copy(x32, x_v, sems.at[3])
    cp_o = pltpu.make_async_copy(wo_hbm.bitcast(U32), wo_v, sems.at[4])
    cp_b = [pltpu.make_async_copy(s_.bitcast(U32), d_, sems.at[5 + i])
            for i, (s_, d_) in enumerate(
                ((w1_hbm, w1_v), (w2_hbm, w2_v), (w3_hbm, w3_v), (w4_hbm, w4_v)))]

    cp_xpre.start()
    for cp in cp_m0:
        cp.start()

    def fetch_pair(hp):
        for mat, w in enumerate((wq_hbm, wk_hbm, wv_hbm)):
            for par in range(2):
                pltpu.make_async_copy(w.bitcast(U32).at[:, par, hp, :],
                                      wqkv.at[6 * hp + 2 * mat + par], wsem.at[hp]).start()

    AHEAD = 10
    for hp in range(AHEAD):
        fetch_pair(hp)

    cv = c_ref[...].astype(F32)
    silu_c = jnp.broadcast_to(cv * jax.nn.sigmoid(cv), (16, D)).astype(BF16)
    with jax.named_scope('P_wait_xpre'):
        cp_xpre.wait()
    xn = _ln(_bf(xpre[...]).astype(F32).reshape(NSEG * NP, D))
    buf[0:NSEG * NP, :] = xn
    for i, cp in enumerate(cp_m0):
        with jax.named_scope('P_wait_m0'):
            cp.wait()
        mod_v[:, i * MC:(i + 1) * MC] = _dot(silu_c, _bf(wmod_v[:, i * MC:(i + 1) * MC]))[0:8]
    sa = mod_v[0:1, 0:D]
    ca1 = 1.0 + mod_v[0:1, D:2 * D]
    hpre[...] = _words(buf[0:NSEG * NP, :] * ca1 + sa)

    def pre_body(hp, _):
        @pl.when(hp == 3)
        def _():
            for later in range(AHEAD, HP):
                fetch_pair(later)
            for cp in [cp_x, cp_o, cp_m1] + cp_b:
                cp.start()

        slabs = wqkv.at[pl.ds(6 * hp, 6)]
        pltpu.make_async_copy(slabs, slabs, wsem.at[hp]).wait()
        for mat in range(3):
            we = wqkv[6 * hp + 2 * mat]
            wo_ = wqkv[6 * hp + 2 * mat + 1]
            w0 = (we & 0xFFFF) | (wo_ << 16)
            w1 = (we >> 16) | (wo_ & np.uint32(0xFFFF0000))
            wqkv[6 * hp + 2 * mat] = w0
            wqkv[6 * hp + 2 * mat + 1] = w1
            lhs = _bf(hpre[...])
            a = _dot(lhs, _bf(w0)).reshape(NSEG, NP, DH)
            b = _dot(lhs, _bf(w1)).reshape(NSEG, NP, DH)
            pre[3 * hp + mat] = _words(
                jnp.concatenate([a, b], axis=1).reshape(NSEG * 2 * NP, DH))

        return 0

    with jax.named_scope("P_pre"):
        jax.lax.fori_loop(0, HP, pre_body, 0)

    def modulated(s):
        return _ln(_bf(x_v[s]).astype(F32)[0:NX]) * ca1 + sa

    cp_x.wait()
    cp_o.wait()
    cp_m1.wait()
    hnext[...] = modulated(0)
    mod_v[:, 2 * D:6 * D] = _dot(silu_c, _bf(wmod_v[:, 2 * D:6 * D]))[0:8]
    ga = mod_v[0:1, 2 * D:3 * D]
    sb = mod_v[0:1, 3 * D:4 * D]
    cb1 = 1.0 + mod_v[0:1, 4 * D:5 * D]
    gb = mod_v[0:1, 5 * D:6 * D]

    def residual(x, att):
        x1 = x + ga * att
        h = _ln(x1) * cb1 + sb
        return x1, h, _ln(h)

    def retire(i):
        x = jnp.concatenate([_bf(x_v[i * SU + u]).astype(F32)[0:NX] for u in range(SU)], axis=0)
        x1, h, hn = residual(x, aprev[...])
        for u in range(SU):
            r = pl.ds(pl.multiple_of((i * SU + u) * SEG, SEG), NX)
            buf[r, :] = x1[u * NX:(u + 1) * NX]
            hbuf[r, :] = h[u * NX:(u + 1) * NX]
        hnl[pl.ds(pl.multiple_of(i * (SU * NX // 2), 8), SU * NX // 2), :] = _words(hn)

    aprev[...] = jnp.zeros((SU * NX, D), F32)

    def seg_step(s, u, mem):
        lhs = jnp.concatenate([mem, hnext[...]], axis=0).astype(BF16)
        hnext[...] = modulated(jnp.minimum(s + 1, NSEG - 1))
        rp = pl.ds(pl.multiple_of(s * NP, NP), NP)
        fill = fill_ref[...]
        vis = fill == 0.0

        def join(mat, hp, a, b):
            ab = jnp.concatenate([a, b], axis=0).astype(BF16)
            return jnp.concatenate([ab, _bf(pre[3 * hp + mat, rp, :])], axis=0)

        def proj(mat, hp):
            j = 6 * hp + 2 * mat
            return join(mat, hp, _dot(lhs, _bf(wqkv[j])), _dot(lhs, _bf(wqkv[j + 1])))

        def probs(q, k):
            sc = jnp.where(vis, _dot_nt(q, k) * scale, fill)
            e = jnp.exp2(sc - jnp.max(sc, axis=-1, keepdims=True))
            den = jnp.sum(e, axis=-1, keepdims=True)
            inv = pl.reciprocal(den, approx=True)
            inv = inv * (2.0 - den * inv)
            return (e * inv).astype(BF16)

        outs = []

        def finish(hp, p, v):
            o = _words(_dot(p, v))
            outs.append(o[0:NL // 2])
            outs.append(o[NL // 2:NL])
            odef[hp, rp, :] = o[NL:]

        def wo_part(h0, h1, j):
            return _dot(_bf(jnp.concatenate(outs[h0:h1], axis=1)),
                        _bf(wo_v[h0 * DH // 2:h1 * DH // 2, j * LANES:(j + 1) * LANES]))

        q, k, v, pr = {}, {}, {}, {}
        js = [2, 3, 0, 1]
        lo = [_dot(lhs[:, :D // 2], _bf(wqkv[j, 0:D // 4, :])) for j in js]
        full = [_dot(lhs[:, D // 2:], _bf(wqkv[j, D // 4:D // 2, :])) + a for a, j in zip(lo, js)]
        k[0] = join(1, 0, full[0], full[1])
        q[0] = join(0, 0, full[2], full[3])
        for hp in range(1, HP):
            k[hp] = proj(1, hp)
            pr[hp - 1] = probs(q[hp - 1], k[hp - 1])
            q[hp] = proj(0, hp)
            if hp >= 2:
                finish(hp - 2, pr[hp - 2], v[hp - 2])
            v[hp - 1] = proj(2, hp - 1)
        half = H // 2
        v[HP - 1] = proj(2, HP - 1)
        pr[HP - 1] = probs(q[HP - 1], k[HP - 1])
        acc = [wo_part(0, half, 0)]
        finish(HP - 2, pr[HP - 2], v[HP - 2])
        acc += [wo_part(0, half, j) for j in range(1, NCT // 2)]
        finish(HP - 1, pr[HP - 1], v[HP - 1])
        acc += [wo_part(0, half, j) for j in range(NCT // 2, NCT)]
        res = jnp.concatenate([wo_part(half, H, j) + acc[j] for j in range(NCT)], axis=1)
        aprev[u * NX:(u + 1) * NX, :] = res[M:]
        return res[:M]

    def seg_body(i, mem):
        retire(jnp.maximum(i - 1, 0))
        for u in range(SU):
            mem = seg_step(i * SU + u, u, mem)
        return mem

    with jax.named_scope("P_seg"):
        jax.lax.fori_loop(0, NSEG // SU, seg_body, mem0_ref[...].astype(F32))
    retire(NSEG // SU - 1)

    for cp in cp_b:
        cp.wait()

    PAD = 8
    ubuf[:, 0:PAD, :] = jnp.zeros((NCT, PAD, LANES), F32)
    ubuf[:, PAD + S:2 * PAD + S, :] = jnp.zeros((NCT, PAD, LANES), F32)

    def stage1(c, _):
        ns = TA // SEG
        rp = pl.ds(pl.multiple_of(c * (ns * NP), ns * NP), ns * NP)
        cols = []
        for hp in range(HP):
            od = _bf(odef[hp, rp, :]).astype(F32).reshape(ns, 2 * NP, DH)
            cols.append(od[:, 0:NP].reshape(ns * NP, DH))
            cols.append(od[:, NP:2 * NP].reshape(ns * NP, DH))
        att = _dot(jnp.concatenate(cols, axis=1).astype(BF16), _bf(wo_v[...]))
        x = _bf(xpre[pl.ds(c * ns, ns)]).astype(F32).reshape(ns * NP, D)
        x1, h, hn = residual(x, att)
        for g in range(ns):
            r = pl.ds(pl.multiple_of(c * TA + g * SEG + NX, 8), NP)
            buf[r, :] = x1[g * NP:(g + 1) * NP]
            hbuf[r, :] = h[g * NP:(g + 1) * NP]
        hl = _bf(hnl[pl.ds(pl.multiple_of(c * (ns * NX // 2), 8), ns * NX // 2), :])
        for lhs, off, n in ((hl, 0, NX), (hn.astype(BF16), NX, NP)):
            u = _gelu(_dot(lhs, _bf(w1_v[...])))
            for j in range(NCT):
                for g in range(ns):
                    ru = pl.ds(pl.multiple_of(c * TA + g * SEG + off + PAD, 8), n)
                    ubuf[j, ru, :] = u[g * n:(g + 1) * n, j * LANES:(j + 1) * LANES]
        return 0

    with jax.named_scope("P_s1"):
        jax.lax.fori_loop(0, S // TA, stage1, 0)

    out32 = out_hbm.bitcast(U32)

    def out_copy(c):
        r = pl.ds(pl.multiple_of(c * (TB // 2), TB // 2), TB // 2)
        return pltpu.make_async_copy(obuf.at[r], out32.at[r], osem.at[c])

    shifts = (-1, 1, -2, 2)

    def stage2(c, _):
        th = TB // 2
        ys = []
        for t in range(2):
            r0 = c * TB + t * th
            g = jnp.concatenate(
                [ubuf[j, pl.ds(r0 + PAD + shifts[j * 4 // NCT], th), :]
                 for j in range(NCT)], axis=1).astype(BF16)
            ys.append(_dot(g, _bf(w2_v[...])) + hbuf[pl.ds(pl.multiple_of(r0, th), th), :])
        yns = [_ln(y).astype(BF16) for y in ys]

        def up(yn, f):
            return _gelu(_dot(yn, _bf(w3_v[:, f * FC:(f + 1) * FC]))).astype(BF16)

        acc = jnp.concatenate(ys, axis=0)
        yn = jnp.concatenate(yns, axis=0)
        t_cur = jnp.concatenate([up(y, 0) for y in yns], axis=0)
        for f in range(FF // FC):
            t_next = up(yn, f + 1) if f + 1 < FF // FC else None
            acc = _dot(t_cur, _bf(w4_v[f * FC // 2:(f + 1) * FC // 2, :])) + acc
            t_cur = t_next
        r = pl.ds(pl.multiple_of(c * TB, TB), TB)
        obuf[pl.ds(pl.multiple_of(c * (TB // 2), TB // 2), TB // 2), :] = _words(
            buf[r, :] + gb * acc)
        out_copy(c).start()
        return 0

    with jax.named_scope("P_s2"):
        jax.lax.fori_loop(0, S // TB, stage2, 0)
    for c in range(S // TB):
        out_copy(c).wait()


@functools.partial(jax.jit, static_argnames=("A_seg_len",))
def pallas_adaLN_cond__memory_aug_recurrent_mem_tr__mixer_s_mlp__prompt_kernel(
    A_x, A_mem0, A_Wq, A_Wk, A_Wv, A_Wo, A_seg_len, B_x, B_w1, B_w2, B_w3, B_w4, c, w_mod,
):
    del B_x
    B, S, D = A_x.shape
    _, H, DH = A_Wq.shape
    M = A_mem0.shape[1]
    SEG = int(A_seg_len)
    FF = B_w3.shape[1]
    assert B == 1 and DH == LANES and M == 8 and SEG == 32 and S % SEG == 0
    NSEG = S // SEG
    NX = NL - M
    NP = SEG - NX
    TB = 128
    SU = 2
    fill = _attn_fill(M, NL, NP)

    hbm = pl.BlockSpec(memory_space=pl.ANY)
    vmem = pl.BlockSpec(memory_space=pltpu.VMEM)
    out = pl.pallas_call(
        functools.partial(_kernel, S=S, D=D, H=H, DH=DH, M=M, SEG=SEG, FF=FF,
                          TA=256, TB=TB, FC=512, SU=SU),
        out_shape=jax.ShapeDtypeStruct((S, D), A_x.dtype),
        in_specs=[hbm, vmem, hbm, hbm, hbm, hbm, hbm, hbm, hbm, hbm, vmem, hbm, vmem],
        out_specs=hbm,
        scratch_shapes=[
            pltpu.VMEM((NSEG, SEG // 2, D), U32),
            pltpu.VMEM((NSEG, NP // 2, D), U32),
            pltpu.VMEM((NSEG * NP // 2, D), U32),
            pltpu.VMEM((NX, D), F32),
            pltpu.VMEM((SU * NX, D), F32),
            pltpu.VMEM((NSEG * NX // 2, D), U32),
            pltpu.VMEM((S, D), F32),
            pltpu.VMEM((3 * H, D // 2, DH), U32),
            pltpu.VMEM((H * DH // 2, D), U32),
            pltpu.VMEM((3 * H // 2, NSEG * NP, DH), U32),
            pltpu.VMEM((H // 2, NSEG * NP, DH), U32),
            pltpu.VMEM((8, 6 * D), F32),
            pltpu.VMEM((D // 2, 6 * D), U32),
            pltpu.VMEM((D // 2, D), U32),
            pltpu.VMEM((D // 2, D), U32),
            pltpu.VMEM((D // 2, FF), U32),
            pltpu.VMEM((FF // 2, D), U32),
            pltpu.VMEM((D // LANES, S + 16, LANES), F32),
            pltpu.VMEM((S, D), F32),
            pltpu.VMEM((S // 2, D), U32),
            pltpu.SemaphoreType.DMA((H // 2,)),
            pltpu.SemaphoreType.DMA((13,)),
            pltpu.SemaphoreType.DMA((S // TB,)),
        ],
        compiler_params=pltpu.CompilerParams(vmem_limit_bytes=127 * 2**20),
        name="adaln_rmt_mixer",
    )(
        A_x.reshape(NSEG, SEG, D), A_mem0.reshape(M, D),
        A_Wq.reshape(D // 2, 2, H, DH), A_Wk.reshape(D // 2, 2, H, DH),
        A_Wv.reshape(D // 2, 2, H, DH),
        A_Wo.reshape(H * DH, D), B_w1, B_w2, B_w3, B_w4, c, w_mod, fill,
    )
    return out.reshape(B, S, D)
```

```python
import functools

import jax
import jax.numpy as jnp
import numpy as np
import jax.experimental.pallas as pl
import jax.experimental.pallas.tpu as pltpu

F32 = jnp.float32
BF16 = jnp.bfloat16
U32 = jnp.uint32
LANES = 128
EPS = 1e-5
LOG2E = 1.4426950408889634
NL = 32


def _ln(x):
    m = jnp.mean(x, axis=-1, keepdims=True)
    d = x - m
    v = jnp.mean(d * d, axis=-1, keepdims=True)
    return d * jax.lax.rsqrt(v + EPS)


def _gelu(x):
    c0 = float(np.sqrt(2.0 / np.pi))
    inner = x * (c0 + (c0 * 0.044715) * (x * x))
    hx = 0.5 * x
    return hx + hx * jnp.tanh(inner)


def _dot(a, b):
    return jnp.dot(a, b, preferred_element_type=F32)


def _dot_nt(a, b):
    return jax.lax.dot_general(a, b, (((1,), (1,)), ((), ())),
                               preferred_element_type=F32)


def _bf(words):
    return pltpu.bitcast(words, BF16)


def _words(x):
    return pltpu.bitcast(x.astype(BF16), U32)


def _st_lhs(a11, a12, a21, a22):
    return [v.astype(BF16) for v in
            (a11 + a22, a21 + a22, a11, a22, a11 + a12, a21 - a11, a12 - a22)]


def _st_rhs(b11, b12, b21, b22):
    return b11 + b22, b12 - b22, b21 - b11, b11 + b12, b21 + b22


def _st_out(m1, m2, m3, m4, m5, m6, m7):
    return (m1 + m4) + (m7 - m5), m3 + m5, m2 + m4, (m1 - m2) + (m3 + m6)


def _attn_fill(n_mem, n_loop, n_pre):
    head = np.concatenate([np.zeros(n_loop), np.ones(n_loop),
                           np.zeros(n_pre), np.ones(n_pre)])
    tok = np.concatenate([np.arange(n_loop), np.arange(n_loop),
                          n_loop + np.arange(n_pre), n_loop + np.arange(n_pre)])
    same = head[:, None] == head[None, :]
    vis = (tok[:, None] < n_mem) | (tok[:, None] >= tok[None, :])
    fill = np.where(same, np.where(vis, 0.0, -1e9 * LOG2E), -np.inf)
    return fill.astype(np.float32)


def _kernel(x_hbm, mem0_ref, wq_hbm, wk_hbm, wv_hbm, wo_hbm, w1_hbm, w2_hbm, w3_hbm,
            w4_hbm, c_ref, wmod_hbm, fill_ref, out_hbm,
            x_v, xpre, hpre, hnext, aprev, hnl, buf, wqkv, wo_v, pre, odef, mod_v, wmod_v,
            w1_v, w2_v, w3_v, w4_v, w3_x, w4_x, ubuf, hbuf, wsem, sems, osem,
            *, S, D, H, DH, M, SEG, FF, TA, TB, FC, SU):
    NSEG = S // SEG
    NX = NL - M
    NP = SEG - NX
    HP = H // 2
    NCT = D // LANES
    scale = float(DH) ** -0.5 * LOG2E

    x32 = x_hbm.bitcast(U32)
    wmod32 = wmod_hbm.bitcast(U32)
    cp_xpre = pltpu.make_async_copy(x32.at[:, pl.ds(NX // 2, NP // 2), :], xpre, sems.at[0])
    MC = D // 2
    cp_m0 = [pltpu.make_async_copy(wmod32.at[:, pl.ds(i * MC, MC)],
                                   wmod_v.at[:, pl.ds(i * MC, MC)], sems.at[9 + i])
             for i in range(2 * D // MC)]
    cp_m1 = pltpu.make_async_copy(wmod32.at[:, pl.ds(2 * D, 4 * D)],
                                  wmod_v.at[:, pl.ds(2 * D, 4 * D)], sems.at[2])
    cp_x = pltpu.make_async_copy(x32, x_v, sems.at[3])
    cp_o = pltpu.make_async_copy(wo_hbm.bitcast(U32), wo_v, sems.at[4])
    cp_b = [pltpu.make_async_copy(s_.bitcast(U32), d_, sems.at[5 + i])
            for i, (s_, d_) in enumerate(
                ((w1_hbm, w1_v), (w2_hbm, w2_v), (w3_hbm, w3_v), (w4_hbm, w4_v)))]

    cp_xpre.start()
    for cp in cp_m0:
        cp.start()

    def fetch_pair(hp):
        for mat, w in enumerate((wq_hbm, wk_hbm, wv_hbm)):
            for par in range(2):
                pltpu.make_async_copy(w.bitcast(U32).at[:, par, hp, :],
                                      wqkv.at[6 * hp + 2 * mat + par], wsem.at[hp]).start()

    AHEAD = 10
    for hp in range(AHEAD):
        fetch_pair(hp)

    cv = c_ref[...].astype(F32)
    silu_c = jnp.broadcast_to(cv * jax.nn.sigmoid(cv), (16, D)).astype(BF16)
    with jax.named_scope('P_wait_xpre'):
        cp_xpre.wait()
    xn = _ln(_bf(xpre[...]).astype(F32).reshape(NSEG * NP, D))
    buf[0:NSEG * NP, :] = xn
    for i, cp in enumerate(cp_m0):
        with jax.named_scope('P_wait_m0'):
            cp.wait()
        mod_v[:, i * MC:(i + 1) * MC] = _dot(silu_c, _bf(wmod_v[:, i * MC:(i + 1) * MC]))[0:8]
    sa = mod_v[0:1, 0:D]
    ca1 = 1.0 + mod_v[0:1, D:2 * D]
    hpre[...] = _words(buf[0:NSEG * NP, :] * ca1 + sa)

    def pre_body(hp, _):
        @pl.when(hp == 3)
        def _():
            for later in range(AHEAD, HP):
                fetch_pair(later)
            for cp in [cp_x, cp_o, cp_m1] + cp_b:
                cp.start()

        slabs = wqkv.at[pl.ds(6 * hp, 6)]
        pltpu.make_async_copy(slabs, slabs, wsem.at[hp]).wait()
        for mat in range(3):
            we = wqkv[6 * hp + 2 * mat]
            wo_ = wqkv[6 * hp + 2 * mat + 1]
            w0 = (we & 0xFFFF) | (wo_ << 16)
            w1 = (we >> 16) | (wo_ & np.uint32(0xFFFF0000))
            wqkv[6 * hp + 2 * mat] = w0
            wqkv[6 * hp + 2 * mat + 1] = w1
            lhs = _bf(hpre[...])
            a = _dot(lhs, _bf(w0)).reshape(NSEG, NP, DH)
            b = _dot(lhs, _bf(w1)).reshape(NSEG, NP, DH)
            pre[3 * hp + mat] = _words(
                jnp.concatenate([a, b], axis=1).reshape(NSEG * 2 * NP, DH))

        return 0

    with jax.named_scope("P_pre"):
        jax.lax.fori_loop(0, HP, pre_body, 0)

    def modulated(s):
        return _ln(_bf(x_v[s]).astype(F32)[0:NX]) * ca1 + sa

    cp_x.wait()
    cp_o.wait()
    cp_m1.wait()
    hnext[...] = modulated(0)
    mod_v[:, 2 * D:6 * D] = _dot(silu_c, _bf(wmod_v[:, 2 * D:6 * D]))[0:8]
    ga = mod_v[0:1, 2 * D:3 * D]
    sb = mod_v[0:1, 3 * D:4 * D]
    cb1 = 1.0 + mod_v[0:1, 4 * D:5 * D]
    gb = mod_v[0:1, 5 * D:6 * D]

    def residual(x, att):
        x1 = x + ga * att
        h = _ln(x1) * cb1 + sb
        return x1, h, _ln(h)

    def retire(i):
        x = jnp.concatenate([_bf(x_v[i * SU + u]).astype(F32)[0:NX] for u in range(SU)], axis=0)
        x1, h, hn = residual(x, aprev[...])
        for u in range(SU):
            r = pl.ds(pl.multiple_of((i * SU + u) * SEG, SEG), NX)
            buf[r, :] = x1[u * NX:(u + 1) * NX]
            hbuf[r, :] = h[u * NX:(u + 1) * NX]
        hnl[pl.ds(pl.multiple_of(i * (SU * NX // 2), 8), SU * NX // 2), :] = _words(hn)

    aprev[...] = jnp.zeros((SU * NX, D), F32)

    def seg_step(s, u, mem):
        lhs = jnp.concatenate([mem, hnext[...]], axis=0).astype(BF16)
        hnext[...] = modulated(jnp.minimum(s + 1, NSEG - 1))
        rp = pl.ds(pl.multiple_of(s * NP, NP), NP)
        fill = fill_ref[...]
        vis = fill == 0.0

        def join(mat, hp, a, b):
            ab = jnp.concatenate([a, b], axis=0).astype(BF16)
            return jnp.concatenate([ab, _bf(pre[3 * hp + mat, rp, :])], axis=0)

        def proj(mat, hp):
            j = 6 * hp + 2 * mat
            return join(mat, hp, _dot(lhs, _bf(wqkv[j])), _dot(lhs, _bf(wqkv[j + 1])))

        def probs(q, k):
            sc = jnp.where(vis, _dot_nt(q, k) * scale, fill)
            e = jnp.exp2(sc - jnp.max(sc, axis=-1, keepdims=True))
            den = jnp.sum(e, axis=-1, keepdims=True)
            inv = pl.reciprocal(den, approx=True)
            inv = inv * (2.0 - den * inv)
            return (e * inv).astype(BF16)

        outs = []

        def finish(hp, p, v):
            o = _words(_dot(p, v))
            outs.append(o[0:NL // 2])
            outs.append(o[NL // 2:NL])
            odef[hp, rp, :] = o[NL:]

        def wo_part(h0, h1, j):
            return _dot(_bf(jnp.concatenate(outs[h0:h1], axis=1)),
                        _bf(wo_v[h0 * DH // 2:h1 * DH // 2, j * LANES:(j + 1) * LANES]))

        q, k, v, pr = {}, {}, {}, {}
        js = [2, 3, 0, 1]
        lo = [_dot(lhs[:, :D // 2], _bf(wqkv[j, 0:D // 4, :])) for j in js]
        full = [_dot(lhs[:, D // 2:], _bf(wqkv[j, D // 4:D // 2, :])) + a for a, j in zip(lo, js)]
        k[0] = join(1, 0, full[0], full[1])
        q[0] = join(0, 0, full[2], full[3])
        for hp in range(1, HP):
            k[hp] = proj(1, hp)
            pr[hp - 1] = probs(q[hp - 1], k[hp - 1])
            q[hp] = proj(0, hp)
            if hp >= 2:
                finish(hp - 2, pr[hp - 2], v[hp - 2])
            v[hp - 1] = proj(2, hp - 1)
        half = H // 2
        v[HP - 1] = proj(2, HP - 1)
        pr[HP - 1] = probs(q[HP - 1], k[HP - 1])
        acc = [wo_part(0, half, 0)]
        finish(HP - 2, pr[HP - 2], v[HP - 2])
        acc += [wo_part(0, half, j) for j in range(1, NCT // 2)]
        finish(HP - 1, pr[HP - 1], v[HP - 1])
        acc += [wo_part(0, half, j) for j in range(NCT // 2, NCT)]
        res = jnp.concatenate([wo_part(half, H, j) + acc[j] for j in range(NCT)], axis=1)
        aprev[u * NX:(u + 1) * NX, :] = res[M:]
        return res[:M]

    def seg_body(i, mem):
        retire(jnp.maximum(i - 1, 0))
        for u in range(SU):
            mem = seg_step(i * SU + u, u, mem)
        return mem

    with jax.named_scope("P_seg"):
        jax.lax.fori_loop(0, NSEG // SU, seg_body, mem0_ref[...].astype(F32))
    retire(NSEG // SU - 1)

    for cp in cp_b:
        cp.wait()

    PAD = 8
    ubuf[:, 0:PAD, :] = jnp.zeros((NCT, PAD, LANES), F32)
    ubuf[:, PAD + S:2 * PAD + S, :] = jnp.zeros((NCT, PAD, LANES), F32)

    DK = D // 2
    FK = FF // 2

    def combine(w_v, extra, c, n):
        kr, kc = w_v.shape[0] // 2, w_v.shape[1] // 2
        rows = kr // n
        for r in range(0, rows, 8):
            r1 = pl.ds(pl.multiple_of(c * rows + r, 8), 8)
            r2 = pl.ds(pl.multiple_of(kr + c * rows + r, 8), 8)
            for j in range(0, kc, 2 * LANES):
                c1, c2 = slice(j, j + 2 * LANES), slice(kc + j, kc + j + 2 * LANES)
                blocks = [_bf(w_v[r_, c_]).astype(F32) for r_ in (r1, r2) for c_ in (c1, c2)]
                q1, q3, q4, q6, q7 = (_words(v) for v in _st_rhs(*blocks))
                w_v[r1, c2] = q3
                w_v[r2, c1] = q4
                extra[0, r1, c1] = q1
                extra[1, r1, c1] = q6
                extra[2, r1, c1] = q7

    def rhs(w_v, extra, r0, nr, c0, nc):
        kr, kc = w_v.shape[0] // 2, w_v.shape[1] // 2
        ra, rb = slice(r0, r0 + nr), slice(kr + r0, kr + r0 + nr)
        ca, cb = slice(c0, c0 + nc), slice(kc + c0, kc + c0 + nc)
        return [lambda: extra[0, ra, ca], lambda: w_v[ra, ca], lambda: w_v[ra, cb],
                lambda: w_v[rb, ca], lambda: w_v[rb, cb], lambda: extra[1, ra, ca],
                lambda: extra[2, ra, ca]]

    def stage1(c, _):
        combine(w3_v, w3_x, c, S // TA)
        combine(w4_v, w4_x, c, S // TA)
        ns = TA // SEG
        rp = pl.ds(pl.multiple_of(c * (ns * NP), ns * NP), ns * NP)
        cols = []
        for hp in range(HP):
            od = _bf(odef[hp, rp, :]).astype(F32).reshape(ns, 2 * NP, DH)
            cols.append(od[:, 0:NP].reshape(ns * NP, DH))
            cols.append(od[:, NP:2 * NP].reshape(ns * NP, DH))
        att = _dot(jnp.concatenate(cols, axis=1).astype(BF16), _bf(wo_v[...]))
        x = _bf(xpre[pl.ds(c * ns, ns)]).astype(F32).reshape(ns * NP, D)
        x1, h, hn = residual(x, att)
        for g in range(ns):
            r = pl.ds(pl.multiple_of(c * TA + g * SEG + NX, 8), NP)
            buf[r, :] = x1[g * NP:(g + 1) * NP]
            hbuf[r, :] = h[g * NP:(g + 1) * NP]
        hl = _bf(hnl[pl.ds(pl.multiple_of(c * (ns * NX // 2), 8), ns * NX // 2), :])
        for lhs, off, n in ((hl, 0, NX), (hn.astype(BF16), NX, NP)):
            u = _gelu(_dot(lhs, _bf(w1_v[...])))
            for j in range(NCT):
                for g in range(ns):
                    ru = pl.ds(pl.multiple_of(c * TA + g * SEG + off + PAD, 8), n)
                    ubuf[j, ru, :] = u[g * n:(g + 1) * n, j * LANES:(j + 1) * LANES]
        return 0

    with jax.named_scope("P_s1"):
        jax.lax.fori_loop(0, S // TA, stage1, 0)

    out32 = out_hbm.bitcast(U32)

    def out_copy(c):
        r = pl.ds(c * (TB // SEG), TB // SEG)
        return pltpu.make_async_copy(x_v.at[r], out32.at[r], osem.at[c])

    shifts = (-1, 1, -2, 2)

    def stage2(c, _):
        th = TB // 2
        ys = []
        for t in range(2):
            r0 = c * TB + t * th
            g = jnp.concatenate(
                [ubuf[j, pl.ds(r0 + PAD + shifts[j * 4 // NCT], th), :]
                 for j in range(NCT)], axis=1).astype(BF16)
            ys.append(_dot(g, _bf(w2_v[...])) + hbuf[pl.ds(pl.multiple_of(r0, th), th), :])
        na, nb = (_ln(y) for y in ys)
        lhs = _st_lhs(na[:, :DK], na[:, DK:], nb[:, :DK], nb[:, DK:])

        def up(j):
            w = rhs(w3_v, w3_x, 0, DK // 2, j * LANES, LANES)
            ms = {i: _dot(lhs[i], _bf(w[i]())) for i in (2, 4, 0, 3, 6, 1, 5)}
            return _st_lhs(*(_gelu(v) for v in _st_out(*(ms[i] for i in range(7)))))

        edges = list(range(0, FK // LANES, FC // LANES)) + [FK // LANES]
        groups = list(zip(edges[:-1], edges[1:]))
        ups = {}
        ms = [None] * 7
        for j0, j1 in groups:
            for j in range(j0, min(j1 + 1, FK // LANES)):
                if j not in ups:
                    ups[j] = up(j)
            w = rhs(w4_v, w4_x, j0 * LANES // 2, (j1 - j0) * LANES // 2, 0, DK)
            for i in range(7):
                t = jnp.concatenate([ups[j][i] for j in range(j0, j1)], axis=1)
                d = _dot(t, _bf(w[i]()))
                ms[i] = d if ms[i] is None else d + ms[i]
        z11, z12, z21, z22 = _st_out(*ms)
        acc = jnp.concatenate(ys, axis=0) + jnp.concatenate(
            [jnp.concatenate([z11, z12], axis=1), jnp.concatenate([z21, z22], axis=1)], axis=0)
        r = pl.ds(pl.multiple_of(c * TB, TB), TB)
        x_v[pl.ds(c * (TB // SEG), TB // SEG)] = _words(buf[r, :] + gb * acc).reshape(
            TB // SEG, SEG // 2, D)
        out_copy(c).start()
        return 0

    with jax.named_scope("P_s2"):
        jax.lax.fori_loop(0, S // TB, stage2, 0)
    for c in range(S // TB):
        out_copy(c).wait()


@functools.partial(jax.jit, static_argnames=("A_seg_len",))
def pallas_adaLN_cond__memory_aug_recurrent_mem_tr__mixer_s_mlp__prompt_kernel(
    A_x, A_mem0, A_Wq, A_Wk, A_Wv, A_Wo, A_seg_len, B_x, B_w1, B_w2, B_w3, B_w4, c, w_mod,
):
    del B_x
    B, S, D = A_x.shape
    _, H, DH = A_Wq.shape
    M = A_mem0.shape[1]
    SEG = int(A_seg_len)
    FF = B_w3.shape[1]
    assert B == 1 and DH == LANES and M == 8 and SEG == 32 and S % SEG == 0
    NSEG = S // SEG
    NX = NL - M
    NP = SEG - NX
    TB = 128
    SU = 2
    fill = _attn_fill(M, NL, NP)

    hbm = pl.BlockSpec(memory_space=pl.ANY)
    vmem = pl.BlockSpec(memory_space=pltpu.VMEM)
    out = pl.pallas_call(
        functools.partial(_kernel, S=S, D=D, H=H, DH=DH, M=M, SEG=SEG, FF=FF,
                          TA=256, TB=TB, FC=512, SU=SU),
        out_shape=jax.ShapeDtypeStruct((NSEG, SEG, D), A_x.dtype),
        in_specs=[hbm, vmem, hbm, hbm, hbm, hbm, hbm, hbm, hbm, hbm, vmem, hbm, vmem],
        out_specs=hbm,
        scratch_shapes=[
            pltpu.VMEM((NSEG, SEG // 2, D), U32),
            pltpu.VMEM((NSEG, NP // 2, D), U32),
            pltpu.VMEM((NSEG * NP // 2, D), U32),
            pltpu.VMEM((NX, D), F32),
            pltpu.VMEM((SU * NX, D), F32),
            pltpu.VMEM((NSEG * NX // 2, D), U32),
            pltpu.VMEM((S, D), F32),
            pltpu.VMEM((3 * H, D // 2, DH), U32),
            pltpu.VMEM((H * DH // 2, D), U32),
            pltpu.VMEM((3 * H // 2, NSEG * NP, DH), U32),
            pltpu.VMEM((H // 2, NSEG * NP, DH), U32),
            pltpu.VMEM((8, 6 * D), F32),
            pltpu.VMEM((D // 2, 6 * D), U32),
            pltpu.VMEM((D // 2, D), U32),
            pltpu.VMEM((D // 2, D), U32),
            pltpu.VMEM((D // 2, FF), U32),
            pltpu.VMEM((FF // 2, D), U32),
            pltpu.VMEM((3, D // 4, FF // 2), U32),
            pltpu.VMEM((3, FF // 4, D // 2), U32),
            pltpu.VMEM((D // LANES, S + 16, LANES), F32),
            pltpu.VMEM((S, D), F32),
            pltpu.SemaphoreType.DMA((H // 2,)),
            pltpu.SemaphoreType.DMA((13,)),
            pltpu.SemaphoreType.DMA((S // TB,)),
        ],
        compiler_params=pltpu.CompilerParams(vmem_limit_bytes=127 * 2**20),
        name="adaln_rmt_mixer",
    )(
        A_x.reshape(NSEG, SEG, D), A_mem0.reshape(M, D),
        A_Wq.reshape(D // 2, 2, H, DH), A_Wk.reshape(D // 2, 2, H, DH),
        A_Wv.reshape(D // 2, 2, H, DH),
        A_Wo.reshape(H * DH, D), B_w1, B_w2, B_w3, B_w4, c, w_mod, fill,
    )
    return out.reshape(B, S, D)
```

```python
import functools

import jax
import jax.numpy as jnp
import numpy as np
import jax.experimental.pallas as pl
import jax.experimental.pallas.tpu as pltpu

F32 = jnp.float32
BF16 = jnp.bfloat16
U32 = jnp.uint32
LANES = 128
EPS = 1e-5
LOG2E = 1.4426950408889634
NL = 32
SU = 2
TA = 256
TC = 256
TB = 128
FG = 4


def _ln(x):
    m = jnp.mean(x, axis=-1, keepdims=True)
    d = x - m
    v = jnp.mean(d * d, axis=-1, keepdims=True)
    return d * jax.lax.rsqrt(v + EPS)


def _gelu(x):
    c0 = float(np.sqrt(2.0 / np.pi))
    inner = x * (c0 + (c0 * 0.044715) * (x * x))
    hx = 0.5 * x
    return hx + hx * jnp.tanh(inner)


def _dot(a, b):
    return jnp.dot(a, b, preferred_element_type=F32)


def _dot_nt(a, b):
    return jax.lax.dot_general(a, b, (((1,), (1,)), ((), ())),
                               preferred_element_type=F32)


def _bf(words):
    return pltpu.bitcast(words, BF16)


def _words(x):
    return pltpu.bitcast(x.astype(BF16), U32)


def _rows(start, n):
    return pl.ds(pl.multiple_of(start, 8), n)


def _st_lhs(a11, a12, a21, a22):
    return [v.astype(BF16) for v in
            (a11 + a22, a21 + a22, a11, a22, a11 + a12, a21 - a11, a12 - a22)]


def _st_rhs(b11, b12, b21, b22):
    b11, b12, b21, b22 = (b.astype(F32) for b in (b11, b12, b21, b22))
    return b11 + b22, b12 - b22, b21 - b11, b11 + b12, b21 + b22


def _st_out(m1, m2, m3, m4, m5, m6, m7):
    return (m1 + m4) + (m7 - m5), m3 + m5, m2 + m4, (m1 - m2) + (m3 + m6)


def _st_matmul(lhs, rhs):
    m2 = _dot(lhs(1), rhs(1))
    m4 = _dot(lhs(3), rhs(3))
    m1 = _dot(lhs(0), rhs(0))
    c21, c11, c22 = m2 + m4, m1 + m4, m1 - m2
    c11 = _dot(lhs(6), rhs(6)) + c11
    m5 = _dot(lhs(4), rhs(4))
    m3 = _dot(lhs(2), rhs(2))
    return c11 - m5, m3 + m5, c21, _dot(lhs(5), rhs(5)) + (c22 + m3)


def _st_store_lhs(dst, r, top, bottom):
    k = top.shape[1] // 2
    for i, v in enumerate(_st_lhs(top[:, :k], top[:, k:], bottom[:, :k], bottom[:, k:])):
        dst[i, r // 2:r // 2 + 8, :] = _words(v)


def _st_prepare(w_v, extra, part, parts):
    kr, kc = w_v.shape[0] // 2, w_v.shape[1] // 2
    rows = kr // parts
    for r in range(0, rows, 8):
        r1, r2 = _rows(part * rows + r, 8), _rows(kr + part * rows + r, 8)
        for j in range(0, kc, 2 * LANES):
            c1, c2 = slice(j, j + 2 * LANES), slice(kc + j, kc + j + 2 * LANES)
            q1, q3, q4, q6, q7 = (_words(v) for v in _st_rhs(
                *(_bf(w_v[r_, c_]) for r_ in (r1, r2) for c_ in (c1, c2))))
            w_v[r1, c2] = q3
            w_v[r2, c1] = q4
            extra[0, r1, c1] = q1
            extra[1, r1, c1] = q6
            extra[2, r1, c1] = q7


def _st_weights(w_v, extra, k0, nk, c0, nc):
    kr, kc = w_v.shape[0] // 2, w_v.shape[1] // 2
    ra, rb = slice(k0 // 2, (k0 + nk) // 2), slice(kr + k0 // 2, kr + (k0 + nk) // 2)
    ca, cb = slice(c0, c0 + nc), slice(kc + c0, kc + c0 + nc)
    where = ((extra, 0, ra, ca), (w_v, ra, ca), (w_v, ra, cb), (w_v, rb, ca),
             (w_v, rb, cb), (extra, 1, ra, ca), (extra, 2, ra, ca))
    return lambda i: _bf(where[i][0][where[i][1:]])


def _attn_fill(n_mem, n_loop, n_pre):
    head = np.concatenate([np.zeros(n_loop), np.ones(n_loop),
                           np.zeros(n_pre), np.ones(n_pre)])
    tok = np.concatenate([np.arange(n_loop), np.arange(n_loop),
                          n_loop + np.arange(n_pre), n_loop + np.arange(n_pre)])
    same = head[:, None] == head[None, :]
    vis = (tok[:, None] < n_mem) | (tok[:, None] >= tok[None, :])
    fill = np.where(same, np.where(vis, 0.0, -1e9 * LOG2E), -np.inf)
    return fill.astype(np.float32)


def _kernel(x_hbm, mem0_ref, wq_hbm, wk_hbm, wv_hbm, wo_hbm, w1_hbm, w2_hbm, w3_hbm,
            w4_hbm, c_ref, wmod_hbm, fill_ref, out_hbm,
            x_v, xpre, x1buf, hbuf, hnl, wo_v, odef, mod_v, w1_v, w2_v, w3_v, w4_v, sems,
            *, S, D, H, DH, M, SEG, FF):
    NSEG = S // SEG
    NX = NL - M
    NP = SEG - NX
    HP = H // 2
    NCT = D // LANES
    DK = D // 2
    scale = float(DH) ** -0.5 * LOG2E

    def mod(i):
        return mod_v[0:1, i * D:(i + 1) * D]

    def residual(x, att):
        x1 = x + mod(2) * att
        h = _ln(x1) * (1.0 + mod(4)) + mod(3)
        return x1, h, _ln(h)

    cp_b = [pltpu.make_async_copy(s_.bitcast(U32), d_, sems.at[i])
            for i, (s_, d_) in enumerate(
                ((w1_hbm, w1_v), (w2_hbm, w2_v), (w3_hbm, w3_v), (w4_hbm, w4_v)))]

    def attention(wqkv, pre, hnext, aprev, wmod_v, hpre, wsem, msem):
        x32 = x_hbm.bitcast(U32)
        wmod32 = wmod_hbm.bitcast(U32)
        cp_xpre = pltpu.make_async_copy(x32.at[:, pl.ds(NX // 2, NP // 2), :], xpre, sems.at[4])
        cp_x = pltpu.make_async_copy(x32, x_v, sems.at[5])
        cp_o = pltpu.make_async_copy(wo_hbm.bitcast(U32), wo_v, sems.at[6])
        mcols = [(i * DK, DK) for i in range(4)] + [(2 * D, 4 * D)]
        cp_m = [pltpu.make_async_copy(wmod32.at[:, pl.ds(a, n)], wmod_v.at[:, pl.ds(a, n)],
                                      msem.at[i]) for i, (a, n) in enumerate(mcols)]

        def fetch_pair(hp):
            for mat, w in enumerate((wq_hbm, wk_hbm, wv_hbm)):
                for par in range(2):
                    pltpu.make_async_copy(w.bitcast(U32).at[:, par, hp, :],
                                          wqkv.at[6 * hp + 2 * mat + par], wsem.at[hp]).start()

        first_pairs = 10
        cp_xpre.start()
        for cp in cp_m[:-1]:
            cp.start()
        for hp in range(first_pairs):
            fetch_pair(hp)

        cv = c_ref[...].astype(F32)
        silu_c = jnp.broadcast_to(cv * jax.nn.sigmoid(cv), (16, D)).astype(BF16)

        def modulation(i):
            a, n = mcols[i]
            cp_m[i].wait()
            mod_v[:, a:a + n] = _dot(silu_c, _bf(wmod_v[:, a:a + n]))[0:8]

        cp_xpre.wait()
        x1buf[0:NSEG * NP, :] = _ln(_bf(xpre[...]).astype(F32).reshape(NSEG * NP, D))
        for i in range(len(mcols) - 1):
            modulation(i)
        sa = mod(0)
        ca1 = 1.0 + mod(1)
        RH = NSEG * NP // 2
        for r in range(0, RH, 16):
            _st_store_lhs(hpre, r, x1buf[r:r + 16, :] * ca1 + sa,
                          x1buf[RH + r:RH + r + 16, :] * ca1 + sa)

        def pre_body(hp, _):
            @pl.when(hp == 3)
            def _():
                for later in range(first_pairs, HP):
                    fetch_pair(later)
                for cp in [cp_x, cp_o, cp_m[-1]] + cp_b:
                    cp.start()

            slabs = wqkv.at[pl.ds(6 * hp, 6)]
            pltpu.make_async_copy(slabs, slabs, wsem.at[hp]).wait()
            for mat in range(3):
                even = wqkv[6 * hp + 2 * mat]
                odd = wqkv[6 * hp + 2 * mat + 1]
                w0 = (even & 0xFFFF) | (odd << 16)
                w1 = (even >> 16) | (odd & np.uint32(0xFFFF0000))
                wqkv[6 * hp + 2 * mat] = w0
                wqkv[6 * hp + 2 * mat + 1] = w1
                b11, b21, b12, b22 = (_bf(w[i * DK // 2:(i + 1) * DK // 2])
                                      for w in (w0, w1) for i in range(2))
                q1, q3, q4, q6, q7 = (v.astype(BF16) for v in _st_rhs(b11, b12, b21, b22))
                rhs = (q1, b11, q3, q4, b22, q6, q7)
                cs = _st_matmul(lambda i: _bf(hpre[i]), lambda i: rhs[i])
                for t in range(2):
                    ab = [v.reshape(NSEG // 2, NP, DH) for v in cs[2 * t:2 * t + 2]]
                    pre[3 * hp + mat, t * RH:(t + 1) * RH, :] = _words(
                        jnp.concatenate(ab, axis=1).reshape(2 * RH, DH))
            return 0

        with jax.named_scope("P_pre"):
            jax.lax.fori_loop(0, HP, pre_body, 0)

        def modulated(s):
            return _ln(_bf(x_v[s]).astype(F32)[0:NX]) * ca1 + sa

        def retire(i):
            x = jnp.concatenate(
                [_bf(x_v[i * SU + u]).astype(F32)[0:NX] for u in range(SU)], axis=0)
            x1, h, hn = residual(x, aprev[...])
            for u in range(SU):
                r = _rows((i * SU + u) * SEG, NX)
                x1buf[r, :] = x1[u * NX:(u + 1) * NX]
                hbuf[r, :] = h[u * NX:(u + 1) * NX]
            hnl[_rows(i * (SU * NX // 2), SU * NX // 2), :] = _words(hn)

        cp_x.wait()
        cp_o.wait()
        modulation(len(mcols) - 1)
        hnext[...] = modulated(0)
        aprev[...] = jnp.zeros((SU * NX, D), F32)

        def seg_step(s, u, mem):
            lhs = jnp.concatenate([mem, hnext[...]], axis=0).astype(BF16)
            hnext[...] = modulated(jnp.minimum(s + 1, NSEG - 1))
            rp = _rows(s * NP, NP)
            fill = fill_ref[...]
            vis = fill == 0.0
            outs = []

            def join(mat, hp, a, b):
                ab = jnp.concatenate([a, b], axis=0).astype(BF16)
                return jnp.concatenate([ab, _bf(pre[3 * hp + mat, rp, :])], axis=0)

            def proj(mat, hp):
                j = 6 * hp + 2 * mat
                return join(mat, hp, _dot(lhs, _bf(wqkv[j])), _dot(lhs, _bf(wqkv[j + 1])))

            def probs(q, k):
                sc = jnp.where(vis, _dot_nt(q, k) * scale, fill)
                e = jnp.exp2(sc - jnp.max(sc, axis=-1, keepdims=True))
                den = jnp.sum(e, axis=-1, keepdims=True)
                inv = pl.reciprocal(den, approx=True)
                inv = inv * (2.0 - den * inv)
                return (e * inv).astype(BF16)

            def finish(hp, p, v):
                o = _words(_dot(p, v))
                outs.append(o[0:NL // 2])
                outs.append(o[NL // 2:NL])
                odef[hp, rp, :] = o[NL:]

            def wo_part(h0, h1, j):
                return _dot(_bf(jnp.concatenate(outs[h0:h1], axis=1)),
                            _bf(wo_v[h0 * DH // 2:h1 * DH // 2, j * LANES:(j + 1) * LANES]))

            q, k, v, pr = {}, {}, {}, {}
            js = [2, 3, 0, 1]
            lo = [_dot(lhs[:, :DK], _bf(wqkv[j, 0:DK // 2, :])) for j in js]
            full = [_dot(lhs[:, DK:], _bf(wqkv[j, DK // 2:DK, :])) + a for a, j in zip(lo, js)]
            k[0] = join(1, 0, full[0], full[1])
            q[0] = join(0, 0, full[2], full[3])
            for hp in range(1, HP):
                k[hp] = proj(1, hp)
                pr[hp - 1] = probs(q[hp - 1], k[hp - 1])
                q[hp] = proj(0, hp)
                if hp >= 2:
                    finish(hp - 2, pr[hp - 2], v[hp - 2])
                v[hp - 1] = proj(2, hp - 1)
            v[HP - 1] = proj(2, HP - 1)
            pr[HP - 1] = probs(q[HP - 1], k[HP - 1])
            acc = [wo_part(0, HP, 0)]
            finish(HP - 2, pr[HP - 2], v[HP - 2])
            acc += [wo_part(0, HP, j) for j in range(1, NCT // 2)]
            finish(HP - 1, pr[HP - 1], v[HP - 1])
            acc += [wo_part(0, HP, j) for j in range(NCT // 2, NCT)]
            res = jnp.concatenate([wo_part(HP, H, j) + acc[j] for j in range(NCT)], axis=1)
            aprev[u * NX:(u + 1) * NX, :] = res[M:]
            return res[:M]

        def seg_body(i, mem):
            retire(jnp.maximum(i - 1, 0))
            for u in range(SU):
                mem = seg_step(i * SU + u, u, mem)
            return mem

        with jax.named_scope("P_seg"):
            jax.lax.fori_loop(0, NSEG // SU, seg_body, mem0_ref[...].astype(F32))
        retire(NSEG // SU - 1)

    pl.run_scoped(
        attention,
        pltpu.VMEM((3 * H, D // 2, DH), U32),
        pltpu.VMEM((3 * HP, NSEG * NP, DH), U32),
        pltpu.VMEM((NX, D), F32),
        pltpu.VMEM((SU * NX, D), F32),
        pltpu.VMEM((D // 2, 6 * D), U32),
        pltpu.VMEM((7, NSEG * NP // 4, DK), U32),
        pltpu.SemaphoreType.DMA((HP,)),
        pltpu.SemaphoreType.DMA((5,)))

    def mixer(ubuf, w2_x, w3_x, w4_x, ynext, osem):
        for cp in cp_b:
            cp.wait()
        PAD = 8
        ubuf[:, 0:PAD, :] = jnp.zeros((NCT, PAD, LANES), F32)
        ubuf[:, PAD + S:2 * PAD + S, :] = jnp.zeros((NCT, PAD, LANES), F32)

        def stage1(c, _):
            for w_v, w_x in ((w2_v, w2_x), (w3_v, w3_x), (w4_v, w4_x)):
                _st_prepare(w_v, w_x, c, S // TA)
            ns = TA // SEG
            rp = _rows(c * (ns * NP), ns * NP)
            cols = []
            for hp in range(HP):
                od = _bf(odef[hp, rp, :]).astype(F32).reshape(ns, 2 * NP, DH)
                cols.append(od[:, 0:NP].reshape(ns * NP, DH))
                cols.append(od[:, NP:2 * NP].reshape(ns * NP, DH))
            att = _dot(jnp.concatenate(cols, axis=1).astype(BF16), _bf(wo_v[...]))
            x = _bf(xpre[pl.ds(c * ns, ns)]).astype(F32).reshape(ns * NP, D)
            x1, h, hn = residual(x, att)
            for g in range(ns):
                r = _rows(c * TA + g * SEG + NX, NP)
                x1buf[r, :] = x1[g * NP:(g + 1) * NP]
                hbuf[r, :] = h[g * NP:(g + 1) * NP]
            hl = _bf(hnl[_rows(c * (ns * NX // 2), ns * NX // 2), :])
            for lhs, off, n in ((hl, 0, NX), (hn.astype(BF16), NX, NP)):
                u = _gelu(_dot(lhs, _bf(w1_v[...])))
                for j in range(NCT):
                    for g in range(ns):
                        ubuf[j, _rows(c * TA + g * SEG + off + PAD, n), :] = (
                            u[g * n:(g + 1) * n, j * LANES:(j + 1) * LANES])
            return 0

        with jax.named_scope("P_s1"):
            jax.lax.fori_loop(0, S // TA, stage1, 0)

        def stage2(c, _):
            th = TC // 2
            shifts = (-1, 1, -2, 2)
            top, bottom = (jnp.concatenate(
                [ubuf[j, pl.ds(c * TC + t * th + PAD + shifts[j * 4 // NCT], th), :]
                 for j in range(NCT)], axis=1) for t in range(2))
            lhs = _st_lhs(top[:, :DK], top[:, DK:], bottom[:, :DK], bottom[:, DK:])
            for j in range(0, DK, LANES):
                cs = _st_matmul(lambda i: lhs[i], _st_weights(w2_v, w2_x, 0, DK, j, LANES))
                for i, v in enumerate(cs):
                    r = _rows(c * TC + (i // 2) * th, th)
                    cc = slice((i % 2) * DK + j, (i % 2) * DK + j + LANES)
                    hbuf[r, cc] = hbuf[r, cc] + v
            return 0

        with jax.named_scope("P_s2"):
            jax.lax.fori_loop(0, S // TC, stage2, 0)

        def ffn_input(c):
            for r in range(0, TB // 2, 16):
                _st_store_lhs(ynext.at[c % 2], r, _ln(hbuf[_rows(c * TB + r, 16), :]),
                              _ln(hbuf[_rows(c * TB + TB // 2 + r, 16), :]))

        def out_copy(c):
            r = pl.ds(c * (TB // SEG), TB // SEG)
            return pltpu.make_async_copy(x_v.at[r], out_hbm.bitcast(U32).at[r], osem.at[c])

        def stage3(c, _):
            def up(j):
                cs = _st_matmul(lambda i: _bf(ynext[c % 2, i]),
                                _st_weights(w3_v, w3_x, 0, DK, j * LANES, LANES))
                return _st_lhs(*(_gelu(v) for v in cs))

            nf = FF // 2 // LANES
            edges = [0] + list(range(nf % FG or FG, nf + 1, FG))
            groups = list(zip(edges[:-1], edges[1:]))
            ups = {j: up(j) for j in range(*groups[0])}
            ms = [None] * 7
            for g, (j0, j1) in enumerate(groups):
                if g + 1 < len(groups):
                    ups.update({j: up(j) for j in range(*groups[g + 1])})
                if g + 2 == len(groups):
                    ffn_input(jnp.where(c + 1 < S // TB, c + 1, 0))
                w = _st_weights(w4_v, w4_x, j0 * LANES, (j1 - j0) * LANES, 0, DK)
                for i in range(7):
                    d = _dot(jnp.concatenate([ups[j][i] for j in range(j0, j1)], axis=1), w(i))
                    ms[i] = d if ms[i] is None else d + ms[i]
            z11, z12, z21, z22 = _st_out(*ms)
            z = jnp.concatenate([jnp.concatenate([z11, z12], axis=1),
                                 jnp.concatenate([z21, z22], axis=1)], axis=0)
            r = _rows(c * TB, TB)
            x_v[pl.ds(c * (TB // SEG), TB // SEG)] = _words(
                x1buf[r, :] + mod(5) * (hbuf[r, :] + z)).reshape(TB // SEG, SEG // 2, D)
            out_copy(c).start()
            return 0

        ffn_input(0)
        with jax.named_scope("P_s3"):
            jax.lax.fori_loop(0, S // TB, stage3, 0)
        for c in range(S // TB):
            out_copy(c).wait()

    pl.run_scoped(
        mixer,
        pltpu.VMEM((NCT, S + 16, LANES), F32),
        pltpu.VMEM((3, D // 4, DK), U32),
        pltpu.VMEM((3, D // 4, FF // 2), U32),
        pltpu.VMEM((3, FF // 4, DK), U32),
        pltpu.VMEM((2, 7, TB // 4, DK), U32),
        pltpu.SemaphoreType.DMA((S // TB,)))


@functools.partial(jax.jit, static_argnames=("A_seg_len",))
def pallas_adaLN_cond__memory_aug_recurrent_mem_tr__mixer_s_mlp__prompt_kernel(
    A_x, A_mem0, A_Wq, A_Wk, A_Wv, A_Wo, A_seg_len, B_x, B_w1, B_w2, B_w3, B_w4, c, w_mod,
):
    del B_x
    B, S, D = A_x.shape
    _, H, DH = A_Wq.shape
    M = A_mem0.shape[1]
    SEG = int(A_seg_len)
    FF = B_w3.shape[1]
    assert B == 1 and DH == LANES and M == 8 and SEG == 32 and S % SEG == 0
    NSEG = S // SEG
    NX = NL - M
    NP = SEG - NX

    hbm = pl.BlockSpec(memory_space=pl.ANY)
    vmem = pl.BlockSpec(memory_space=pltpu.VMEM)
    out = pl.pallas_call(
        functools.partial(_kernel, S=S, D=D, H=H, DH=DH, M=M, SEG=SEG, FF=FF),
        out_shape=jax.ShapeDtypeStruct((NSEG, SEG, D), A_x.dtype),
        in_specs=[hbm, vmem, hbm, hbm, hbm, hbm, hbm, hbm, hbm, hbm, vmem, hbm, vmem],
        out_specs=hbm,
        scratch_shapes=[
            pltpu.VMEM((NSEG, SEG // 2, D), U32),
            pltpu.VMEM((NSEG, NP // 2, D), U32),
            pltpu.VMEM((S, D), F32),
            pltpu.VMEM((S, D), F32),
            pltpu.VMEM((NSEG * NX // 2, D), U32),
            pltpu.VMEM((H * DH // 2, D), U32),
            pltpu.VMEM((H // 2, NSEG * NP, DH), U32),
            pltpu.VMEM((8, 6 * D), F32),
            pltpu.VMEM((D // 2, D), U32),
            pltpu.VMEM((D // 2, D), U32),
            pltpu.VMEM((D // 2, FF), U32),
            pltpu.VMEM((FF // 2, D), U32),
            pltpu.SemaphoreType.DMA((7,)),
        ],
        compiler_params=pltpu.CompilerParams(vmem_limit_bytes=124 * 2**20),
        name="adaln_rmt_mixer",
    )(
        A_x.reshape(NSEG, SEG, D), A_mem0.reshape(M, D),
        A_Wq.reshape(D // 2, 2, H, DH), A_Wk.reshape(D // 2, 2, H, DH),
        A_Wv.reshape(D // 2, 2, H, DH),
        A_Wo.reshape(H * DH, D), B_w1, B_w2, B_w3, B_w4, c, w_mod, _attn_fill(M, NL, NP),
    )
    return out.reshape(B, S, D)
```

```python
import functools

import jax
import jax.numpy as jnp
import numpy as np
import jax.experimental.pallas as pl
import jax.experimental.pallas.tpu as pltpu

F32 = jnp.float32
BF16 = jnp.bfloat16
U32 = jnp.uint32
LANES = 128
EPS = 1e-5
LOG2E = 1.4426950408889634
NL = 32
SU = 2
TA = 256
TC = 256
TB = 128
FG = 4


def _ln(x):
    m = jnp.mean(x, axis=-1, keepdims=True)
    d = x - m
    v = jnp.mean(d * d, axis=-1, keepdims=True)
    return d * jax.lax.rsqrt(v + EPS)


def _gelu(x):
    c0 = float(np.sqrt(2.0 / np.pi))
    inner = x * (c0 + (c0 * 0.044715) * (x * x))
    hx = 0.5 * x
    return hx + hx * jnp.tanh(inner)


def _dot(a, b):
    return jnp.dot(a, b, preferred_element_type=F32)


def _dot_nt(a, b):
    return jax.lax.dot_general(a, b, (((1,), (1,)), ((), ())),
                               preferred_element_type=F32)


def _bf(words):
    return pltpu.bitcast(words, BF16)


def _words(x):
    return pltpu.bitcast(x.astype(BF16), U32)


def _rows(start, n):
    return pl.ds(pl.multiple_of(start, 8), n)


def _st_lhs(a11, a12, a21, a22):
    return [v.astype(BF16) for v in
            (a11 + a22, a21 + a22, a11, a22, a11 + a12, a21 - a11, a12 - a22)]


def _st_rhs(b11, b12, b21, b22):
    b11, b12, b21, b22 = (b.astype(F32) for b in (b11, b12, b21, b22))
    return b11 + b22, b12 - b22, b21 - b11, b11 + b12, b21 + b22


def _st_out(m1, m2, m3, m4, m5, m6, m7):
    return (m1 + m4) + (m7 - m5), m3 + m5, m2 + m4, (m1 - m2) + (m3 + m6)


def _st_matmul(lhs, rhs):
    m2 = _dot(lhs(1), rhs(1))
    m4 = _dot(lhs(3), rhs(3))
    m1 = _dot(lhs(0), rhs(0))
    c21, c11, c22 = m2 + m4, m1 + m4, m1 - m2
    c11 = _dot(lhs(6), rhs(6)) + c11
    m5 = _dot(lhs(4), rhs(4))
    m3 = _dot(lhs(2), rhs(2))
    return c11 - m5, m3 + m5, c21, _dot(lhs(5), rhs(5)) + (c22 + m3)


def _st_store_lhs(dst, r, top, bottom):
    k = top.shape[1] // 2
    for i, v in enumerate(_st_lhs(top[:, :k], top[:, k:], bottom[:, :k], bottom[:, k:])):
        dst[i, r // 2:r // 2 + 8, :] = _words(v)


def _st_prepare(w_v, extra, part, parts):
    kr, kc = w_v.shape[0] // 2, w_v.shape[1] // 2
    rows = kr // parts
    for r in range(0, rows, 8):
        r1, r2 = _rows(part * rows + r, 8), _rows(kr + part * rows + r, 8)
        for j in range(0, kc, 2 * LANES):
            c1, c2 = slice(j, j + 2 * LANES), slice(kc + j, kc + j + 2 * LANES)
            q1, q3, q4, q6, q7 = (_words(v) for v in _st_rhs(
                *(_bf(w_v[r_, c_]) for r_ in (r1, r2) for c_ in (c1, c2))))
            w_v[r1, c2] = q3
            w_v[r2, c1] = q4
            extra[0, r1, c1] = q1
            extra[1, r1, c1] = q6
            extra[2, r1, c1] = q7


def _st_weights(w_v, extra, k0, nk, c0, nc):
    kr, kc = w_v.shape[0] // 2, w_v.shape[1] // 2
    ra, rb = slice(k0 // 2, (k0 + nk) // 2), slice(kr + k0 // 2, kr + (k0 + nk) // 2)
    ca, cb = slice(c0, c0 + nc), slice(kc + c0, kc + c0 + nc)
    where = ((extra, 0, ra, ca), (w_v, ra, ca), (w_v, ra, cb), (w_v, rb, ca),
             (w_v, rb, cb), (extra, 1, ra, ca), (extra, 2, ra, ca))
    return lambda i: _bf(where[i][0][where[i][1:]])


def _attn_fill(n_mem, n_loop, n_pre):
    n = 2 * (n_loop + n_pre)

    def head_token(axis):
        i = jax.lax.broadcasted_iota(jnp.int32, (n, n), axis)
        in_loop = i < 2 * n_loop
        second = jnp.where(i >= jnp.where(in_loop, n_loop, 2 * n_loop + n_pre), 1, 0)
        return second, jnp.where(in_loop, i - second * n_loop, i - n_loop - second * n_pre)

    (hq, tq), (hk, tk) = head_token(0), head_token(1)
    causal = jnp.where((tq < n_mem) | (tq >= tk), 0.0, -1e9 * LOG2E)
    return jnp.where(hq == hk, causal, -np.inf).astype(F32)


def _kernel(x_hbm, mem0_hbm, wq_hbm, wk_hbm, wv_hbm, wo_hbm, w1_hbm, w2_hbm, w3_hbm,
            w4_hbm, c_hbm, wmod_hbm, out_hbm,
            x_v, xpre, x1buf, hbuf, hnl, wo_v, odef, mod_v, w1_v, w2_v, w3_v, w4_v, sems,
            *, S, D, H, DH, M, SEG, FF):
    NSEG = S // SEG
    NX = NL - M
    NP = SEG - NX
    HP = H // 2
    NCT = D // LANES
    DK = D // 2
    scale = float(DH) ** -0.5 * LOG2E

    def mod(i):
        return mod_v[0:1, i * D:(i + 1) * D]

    def residual(x, att):
        x1 = x + mod(2) * att
        h = _ln(x1) * (1.0 + mod(4)) + mod(3)
        return x1, h, _ln(h)

    cp_b = [pltpu.make_async_copy(s_.bitcast(U32), d_, sems.at[i])
            for i, (s_, d_) in enumerate(
                ((w1_hbm, w1_v), (w2_hbm, w2_v), (w3_hbm, w3_v), (w4_hbm, w4_v)))]

    def attention(wqkv, pre, hnext, aprev, wmod_v, hpre, c_v, mem0_v, fill_v, wsem, msem):
        x32 = x_hbm.bitcast(U32)
        wmod32 = wmod_hbm.bitcast(U32)
        cp_xpre = pltpu.make_async_copy(x32.at[:, pl.ds(NX // 2, NP // 2), :], xpre, sems.at[4])
        cp_x = pltpu.make_async_copy(x32, x_v, sems.at[5])
        cp_o = pltpu.make_async_copy(wo_hbm.bitcast(U32), wo_v, sems.at[6])
        mcols = [(i * DK, DK) for i in range(4)] + [(2 * D, 4 * D)]
        cp_m = [pltpu.make_async_copy(wmod32.at[:, pl.ds(a, n)], wmod_v.at[:, pl.ds(a, n)],
                                      msem.at[i]) for i, (a, n) in enumerate(mcols)]

        def fetch_pair(hp):
            for mat, w in enumerate((wq_hbm, wk_hbm, wv_hbm)):
                for par in range(2):
                    pltpu.make_async_copy(w.bitcast(U32).at[:, par, hp, :],
                                          wqkv.at[6 * hp + 2 * mat + par], wsem.at[hp]).start()

        cp_c = pltpu.make_async_copy(c_hbm, c_v, sems.at[7])
        cp_mem = pltpu.make_async_copy(mem0_hbm, mem0_v, sems.at[8])
        for cp in [cp_c, cp_mem, cp_xpre] + cp_m[:-1]:
            cp.start()
        fetch_pair(0)
        first_pairs = 10

        fill_v[...] = _attn_fill(M, NL, NP)
        cp_c.wait()
        cp_mem.wait()
        cv = c_v[...].astype(F32)
        silu_c = jnp.broadcast_to(cv * jax.nn.sigmoid(cv), (16, D)).astype(BF16)

        def modulation(i):
            a, n = mcols[i]
            cp_m[i].wait()
            mod_v[:, a:a + n] = _dot(silu_c, _bf(wmod_v[:, a:a + n]))[0:8]

        cp_xpre.wait()
        x1buf[0:NSEG * NP, :] = _ln(_bf(xpre[...]).astype(F32).reshape(NSEG * NP, D))
        for i in range(len(mcols) - 1):
            modulation(i)
        for hp in range(1, first_pairs):
            fetch_pair(hp)
        sa = mod(0)
        ca1 = 1.0 + mod(1)
        RH = NSEG * NP // 2
        for r in range(0, RH, 16):
            _st_store_lhs(hpre, r, x1buf[r:r + 16, :] * ca1 + sa,
                          x1buf[RH + r:RH + r + 16, :] * ca1 + sa)

        def pre_body(hp, _):
            @pl.when(hp == 3)
            def _():
                for later in range(first_pairs, HP):
                    fetch_pair(later)
                for cp in [cp_x, cp_o, cp_m[-1]] + cp_b:
                    cp.start()

            slabs = wqkv.at[pl.ds(6 * hp, 6)]
            pltpu.make_async_copy(slabs, slabs, wsem.at[hp]).wait()
            for mat in range(3):
                even = wqkv[6 * hp + 2 * mat]
                odd = wqkv[6 * hp + 2 * mat + 1]
                w0 = (even & 0xFFFF) | (odd << 16)
                w1 = (even >> 16) | (odd & np.uint32(0xFFFF0000))
                wqkv[6 * hp + 2 * mat] = w0
                wqkv[6 * hp + 2 * mat + 1] = w1
                b11, b21, b12, b22 = (_bf(w[i * DK // 2:(i + 1) * DK // 2])
                                      for w in (w0, w1) for i in range(2))
                q1, q3, q4, q6, q7 = (v.astype(BF16) for v in _st_rhs(b11, b12, b21, b22))
                rhs = (q1, b11, q3, q4, b22, q6, q7)
                cs = _st_matmul(lambda i: _bf(hpre[i]), lambda i: rhs[i])
                for t in range(2):
                    ab = [v.reshape(NSEG // 2, NP, DH) for v in cs[2 * t:2 * t + 2]]
                    pre[3 * hp + mat, t * RH:(t + 1) * RH, :] = _words(
                        jnp.concatenate(ab, axis=1).reshape(2 * RH, DH))
            return 0

        with jax.named_scope("P_pre"):
            jax.lax.fori_loop(0, HP, pre_body, 0)

        def modulated(s):
            return _ln(_bf(x_v[s]).astype(F32)[0:NX]) * ca1 + sa

        def retire(i):
            x = jnp.concatenate(
                [_bf(x_v[i * SU + u]).astype(F32)[0:NX] for u in range(SU)], axis=0)
            x1, h, hn = residual(x, aprev[...])
            for u in range(SU):
                r = _rows((i * SU + u) * SEG, NX)
                x1buf[r, :] = x1[u * NX:(u + 1) * NX]
                hbuf[r, :] = h[u * NX:(u + 1) * NX]
            hnl[_rows(i * (SU * NX // 2), SU * NX // 2), :] = _words(hn)

        cp_x.wait()
        cp_o.wait()
        modulation(len(mcols) - 1)
        hnext[...] = modulated(0)
        aprev[...] = jnp.zeros((SU * NX, D), F32)

        def seg_step(s, u, mem):
            lhs = jnp.concatenate([mem, hnext[...]], axis=0).astype(BF16)
            hnext[...] = modulated(jnp.minimum(s + 1, NSEG - 1))
            rp = _rows(s * NP, NP)
            fill = fill_v[...]
            vis = fill == 0.0
            outs = []

            def join(mat, hp, a, b):
                ab = jnp.concatenate([a, b], axis=0).astype(BF16)
                return jnp.concatenate([ab, _bf(pre[3 * hp + mat, rp, :])], axis=0)

            def proj(mat, hp):
                j = 6 * hp + 2 * mat
                return join(mat, hp, _dot(lhs, _bf(wqkv[j])), _dot(lhs, _bf(wqkv[j + 1])))

            def probs(q, k):
                sc = jnp.where(vis, _dot_nt(q, k) * scale, fill)
                e = jnp.exp2(sc - jnp.max(sc, axis=-1, keepdims=True))
                den = jnp.sum(e, axis=-1, keepdims=True)
                inv = pl.reciprocal(den, approx=True)
                inv = inv * (2.0 - den * inv)
                return (e * inv).astype(BF16)

            def finish(hp, p, v):
                o = _words(_dot(p, v))
                outs.append(o[0:NL // 2])
                outs.append(o[NL // 2:NL])
                odef[hp, rp, :] = o[NL:]

            def wo_part(h0, h1, j):
                return _dot(_bf(jnp.concatenate(outs[h0:h1], axis=1)),
                            _bf(wo_v[h0 * DH // 2:h1 * DH // 2, j * LANES:(j + 1) * LANES]))

            q, k, v, pr = {}, {}, {}, {}
            js = [2, 3, 0, 1]
            lo = [_dot(lhs[:, :DK], _bf(wqkv[j, 0:DK // 2, :])) for j in js]
            full = [_dot(lhs[:, DK:], _bf(wqkv[j, DK // 2:DK, :])) + a for a, j in zip(lo, js)]
            k[0] = join(1, 0, full[0], full[1])
            q[0] = join(0, 0, full[2], full[3])
            for hp in range(1, HP):
                k[hp] = proj(1, hp)
                pr[hp - 1] = probs(q[hp - 1], k[hp - 1])
                q[hp] = proj(0, hp)
                if hp >= 2:
                    finish(hp - 2, pr[hp - 2], v[hp - 2])
                v[hp - 1] = proj(2, hp - 1)
            v[HP - 1] = proj(2, HP - 1)
            pr[HP - 1] = probs(q[HP - 1], k[HP - 1])
            acc = [wo_part(0, HP, 0)]
            finish(HP - 2, pr[HP - 2], v[HP - 2])
            acc += [wo_part(0, HP, j) for j in range(1, NCT // 2)]
            finish(HP - 1, pr[HP - 1], v[HP - 1])
            acc += [wo_part(0, HP, j) for j in range(NCT // 2, NCT)]
            res = jnp.concatenate([wo_part(HP, H, j) + acc[j] for j in range(NCT)], axis=1)
            aprev[u * NX:(u + 1) * NX, :] = res[M:]
            return res[:M]

        def seg_body(i, mem):
            retire(jnp.maximum(i - 1, 0))
            for u in range(SU):
                mem = seg_step(i * SU + u, u, mem)
            return mem

        with jax.named_scope("P_seg"):
            jax.lax.fori_loop(0, NSEG // SU, seg_body, mem0_v[...].astype(F32))
        retire(NSEG // SU - 1)

    pl.run_scoped(
        attention,
        pltpu.VMEM((3 * H, D // 2, DH), U32),
        pltpu.VMEM((3 * HP, NSEG * NP, DH), U32),
        pltpu.VMEM((NX, D), F32),
        pltpu.VMEM((SU * NX, D), F32),
        pltpu.VMEM((D // 2, 6 * D), U32),
        pltpu.VMEM((7, NSEG * NP // 4, DK), U32),
        pltpu.VMEM((1, D), BF16),
        pltpu.VMEM((M, D), BF16),
        pltpu.VMEM((2 * (NL + NP),) * 2, F32),
        pltpu.SemaphoreType.DMA((HP,)),
        pltpu.SemaphoreType.DMA((5,)))

    def mixer(ubuf, w2_x, w3_x, w4_x, ynext, obuf, osem):
        for cp in cp_b:
            cp.wait()
        PAD = 8
        ubuf[:, 0:PAD, :] = jnp.zeros((NCT, PAD, LANES), F32)
        ubuf[:, PAD + S:2 * PAD + S, :] = jnp.zeros((NCT, PAD, LANES), F32)

        def stage1(c, _):
            for w_v, w_x in ((w2_v, w2_x), (w3_v, w3_x), (w4_v, w4_x)):
                _st_prepare(w_v, w_x, c, S // TA)
            ns = TA // SEG
            rp = _rows(c * (ns * NP), ns * NP)
            cols = []
            for hp in range(HP):
                od = _bf(odef[hp, rp, :]).astype(F32).reshape(ns, 2 * NP, DH)
                cols.append(od[:, 0:NP].reshape(ns * NP, DH))
                cols.append(od[:, NP:2 * NP].reshape(ns * NP, DH))
            att = _dot(jnp.concatenate(cols, axis=1).astype(BF16), _bf(wo_v[...]))
            x = _bf(xpre[pl.ds(c * ns, ns)]).astype(F32).reshape(ns * NP, D)
            x1, h, hn = residual(x, att)
            for g in range(ns):
                r = _rows(c * TA + g * SEG + NX, NP)
                x1buf[r, :] = x1[g * NP:(g + 1) * NP]
                hbuf[r, :] = h[g * NP:(g + 1) * NP]
            hl = _bf(hnl[_rows(c * (ns * NX // 2), ns * NX // 2), :])
            for lhs, off, n in ((hl, 0, NX), (hn.astype(BF16), NX, NP)):
                u = _gelu(_dot(lhs, _bf(w1_v[...])))
                for j in range(NCT):
                    for g in range(ns):
                        ubuf[j, _rows(c * TA + g * SEG + off + PAD, n), :] = (
                            u[g * n:(g + 1) * n, j * LANES:(j + 1) * LANES])
            return 0

        with jax.named_scope("P_s1"):
            jax.lax.fori_loop(0, S // TA, stage1, 0)

        def stage2(c, _):
            th = TC // 2
            shifts = (-1, 1, -2, 2)
            top, bottom = (jnp.concatenate(
                [ubuf[j, pl.ds(c * TC + t * th + PAD + shifts[j * 4 // NCT], th), :]
                 for j in range(NCT)], axis=1) for t in range(2))
            lhs = _st_lhs(top[:, :DK], top[:, DK:], bottom[:, :DK], bottom[:, DK:])
            for j in range(0, DK, LANES):
                cs = _st_matmul(lambda i: lhs[i], _st_weights(w2_v, w2_x, 0, DK, j, LANES))
                for i, v in enumerate(cs):
                    r = _rows(c * TC + (i // 2) * th, th)
                    cc = slice((i % 2) * DK + j, (i % 2) * DK + j + LANES)
                    hbuf[r, cc] = hbuf[r, cc] + v
            return 0

        with jax.named_scope("P_s2"):
            jax.lax.fori_loop(0, S // TC, stage2, 0)

        def ffn_input(c, r):
            _st_store_lhs(ynext.at[c % 2], r, _ln(hbuf[_rows(c * TB + r, 16), :]),
                          _ln(hbuf[_rows(c * TB + TB // 2 + r, 16), :]))

        def out_copy(c):
            return pltpu.make_async_copy(obuf.at[c], out_hbm.at[c], osem.at[c])

        def stage3(c, _):
            nf = FF // 2 // LANES
            pieces = list(range(0, TB // 2, 16))
            due = {(i + 1) * (nf - 1) // len(pieces): r for i, r in enumerate(pieces)}

            def up(j):
                if j in due:
                    ffn_input(jnp.where(c + 1 < S // TB, c + 1, 0), due[j])
                cs = _st_matmul(lambda i: _bf(ynext[c % 2, i]),
                                _st_weights(w3_v, w3_x, 0, DK, j * LANES, LANES))
                return [_words(t) for t in _st_lhs(*(_gelu(v) for v in cs))]

            edges = [0] + list(range(nf % FG or FG, nf + 1, FG))
            groups = list(zip(edges[:-1], edges[1:]))
            ups = {j: up(j) for j in range(*groups[0])}
            ms = {}
            for g, (j0, j1) in enumerate(groups):
                if g + 1 < len(groups):
                    ups.update({j: up(j) for j in range(*groups[g + 1])})
                ts = [_bf(jnp.concatenate([ups[j][i] for j in range(j0, j1)], axis=1))
                      for i in range(7)]
                for n in range(0, DK, LANES):
                    w = _st_weights(w4_v, w4_x, j0 * LANES, (j1 - j0) * LANES, n, LANES)
                    for i in range(7):
                        d = _dot(ts[i], w(i))
                        ms[n, i] = d + ms[n, i] if g else d
            for n in range(0, DK, LANES):
                for i, z in enumerate(_st_out(*(ms[n, i] for i in range(7)))):
                    r0 = (i // 2) * (TB // 2)
                    r = _rows(c * TB + r0, TB // 2)
                    cc = slice((i % 2) * DK + n, (i % 2) * DK + n + LANES)
                    obuf[c, r0:r0 + TB // 2, cc] = (
                        x1buf[r, cc] + mod(5)[:, cc] * (hbuf[r, cc] + z)).astype(obuf.dtype)
            out_copy(c).start()
            return 0

        for r in range(0, TB // 2, 16):
            ffn_input(0, r)
        with jax.named_scope("P_s3"):
            jax.lax.fori_loop(0, S // TB, stage3, 0)
        for c in range(S // TB):
            out_copy(c).wait()

    pl.run_scoped(
        mixer,
        pltpu.VMEM((NCT, S + 16, LANES), F32),
        pltpu.VMEM((3, D // 4, DK), U32),
        pltpu.VMEM((3, D // 4, FF // 2), U32),
        pltpu.VMEM((3, FF // 4, DK), U32),
        pltpu.VMEM((2, 7, TB // 4, DK), U32),
        pltpu.VMEM(out_hbm.shape, out_hbm.dtype),
        pltpu.SemaphoreType.DMA((S // TB,)))


@functools.partial(jax.jit, static_argnames=("A_seg_len",))
def pallas_adaLN_cond__memory_aug_recurrent_mem_tr__mixer_s_mlp__prompt_kernel(
    A_x, A_mem0, A_Wq, A_Wk, A_Wv, A_Wo, A_seg_len, B_x, B_w1, B_w2, B_w3, B_w4, c, w_mod,
):
    del B_x
    B, S, D = A_x.shape
    _, H, DH = A_Wq.shape
    M = A_mem0.shape[1]
    SEG = int(A_seg_len)
    FF = B_w3.shape[1]
    assert B == 1 and DH == LANES and M == 8 and SEG == 32 and S % SEG == 0
    NSEG = S // SEG
    NX = NL - M
    NP = SEG - NX

    hbm = pl.BlockSpec(memory_space=pl.ANY)
    out = pl.pallas_call(
        functools.partial(_kernel, S=S, D=D, H=H, DH=DH, M=M, SEG=SEG, FF=FF),
        out_shape=jax.ShapeDtypeStruct((S // TB, TB, D), A_x.dtype),
        in_specs=[hbm] * 12,
        out_specs=hbm,
        scratch_shapes=[
            pltpu.VMEM((NSEG, SEG // 2, D), U32),
            pltpu.VMEM((NSEG, NP // 2, D), U32),
            pltpu.VMEM((S, D), F32),
            pltpu.VMEM((S, D), F32),
            pltpu.VMEM((NSEG * NX // 2, D), U32),
            pltpu.VMEM((H * DH // 2, D), U32),
            pltpu.VMEM((H // 2, NSEG * NP, DH), U32),
            pltpu.VMEM((8, 6 * D), F32),
            pltpu.VMEM((D // 2, D), U32),
            pltpu.VMEM((D // 2, D), U32),
            pltpu.VMEM((D // 2, FF), U32),
            pltpu.VMEM((FF // 2, D), U32),
            pltpu.SemaphoreType.DMA((9,)),
        ],
        compiler_params=pltpu.CompilerParams(vmem_limit_bytes=124 * 2**20),
        name="adaln_rmt_mixer",
    )(
        A_x.reshape(NSEG, SEG, D), A_mem0.reshape(M, D),
        A_Wq.reshape(D // 2, 2, H, DH), A_Wk.reshape(D // 2, 2, H, DH),
        A_Wv.reshape(D // 2, 2, H, DH),
        A_Wo.reshape(H * DH, D), B_w1, B_w2, B_w3, B_w4, c, w_mod,
    )
    return out.reshape(B, S, D)
```

```python
import functools

import jax
import jax.numpy as jnp
import numpy as np
import jax.experimental.pallas as pl
import jax.experimental.pallas.tpu as pltpu

F32 = jnp.float32
BF16 = jnp.bfloat16
U32 = jnp.uint32
LANES = 128
EPS = 1e-5
LOG2E = 1.4426950408889634
NL = 32
PAD = 8
TC = 256
TB = 128
FG = 4


def _ln(x):
    m = jnp.mean(x, axis=-1, keepdims=True)
    d = x - m
    v = jnp.mean(d * d, axis=-1, keepdims=True)
    return d * jax.lax.rsqrt(v + EPS)


def _gelu(x):
    c0 = float(np.sqrt(2.0 / np.pi))
    inner = x * (c0 + (c0 * 0.044715) * (x * x))
    hx = 0.5 * x
    return hx + hx * jnp.tanh(inner)


def _dot(a, b):
    return jnp.dot(a, b, preferred_element_type=F32)


def _dot_nt(a, b):
    return jax.lax.dot_general(a, b, (((1,), (1,)), ((), ())),
                               preferred_element_type=F32)


def _bf(words):
    return pltpu.bitcast(words, BF16)


def _words(x):
    return pltpu.bitcast(x.astype(BF16), U32)


def _rows(start, n):
    return pl.ds(pl.multiple_of(start, 8), n)


def _st_lhs(a11, a12, a21, a22):
    return [v.astype(BF16) for v in
            (a11 + a22, a21 + a22, a11, a22, a11 + a12, a21 - a11, a12 - a22)]


def _st_rhs(b11, b12, b21, b22):
    b11, b12, b21, b22 = (b.astype(F32) for b in (b11, b12, b21, b22))
    return b11 + b22, b12 - b22, b21 - b11, b11 + b12, b21 + b22


def _st_out(m1, m2, m3, m4, m5, m6, m7):
    return (m1 + m4) + (m7 - m5), m3 + m5, m2 + m4, (m1 - m2) + (m3 + m6)


def _st_matmul(lhs, rhs):
    m2 = _dot(lhs(1), rhs(1))
    m4 = _dot(lhs(3), rhs(3))
    m1 = _dot(lhs(0), rhs(0))
    c21, c11, c22 = m2 + m4, m1 + m4, m1 - m2
    c11 = _dot(lhs(6), rhs(6)) + c11
    m5 = _dot(lhs(4), rhs(4))
    m3 = _dot(lhs(2), rhs(2))
    return c11 - m5, m3 + m5, c21, _dot(lhs(5), rhs(5)) + (c22 + m3)


def _st_store_lhs(dst, word_row, top, bottom):
    n, k = top.shape[0] // 2, top.shape[1] // 2
    for i, v in enumerate(_st_lhs(top[:, :k], top[:, k:], bottom[:, :k], bottom[:, k:])):
        dst[i, _rows(word_row, n), :] = _words(v)


def _st_prepare(w_v, extra, part, parts):
    kr, kc = w_v.shape[0] // 2, w_v.shape[1] // 2
    rows = kr // parts
    for r in range(0, rows, 8):
        r1, r2 = _rows(part * rows + r, 8), _rows(kr + part * rows + r, 8)
        for j in range(0, kc, 2 * LANES):
            c1, c2 = slice(j, j + 2 * LANES), slice(kc + j, kc + j + 2 * LANES)
            q1, q3, q4, q6, q7 = (_words(v) for v in _st_rhs(
                *(_bf(w_v[r_, c_]) for r_ in (r1, r2) for c_ in (c1, c2))))
            w_v[r1, c2] = q3
            w_v[r2, c1] = q4
            extra[0, r1, c1] = q1
            extra[1, r1, c1] = q6
            extra[2, r1, c1] = q7


def _st_weights(w_v, extra, k0, nk, c0, nc):
    kr, kc = w_v.shape[0] // 2, w_v.shape[1] // 2
    ra, rb = slice(k0 // 2, (k0 + nk) // 2), slice(kr + k0 // 2, kr + (k0 + nk) // 2)
    ca, cb = slice(c0, c0 + nc), slice(kc + c0, kc + c0 + nc)
    where = ((extra, 0, ra, ca), (w_v, ra, ca), (w_v, ra, cb), (w_v, rb, ca),
             (w_v, rb, cb), (extra, 1, ra, ca), (extra, 2, ra, ca))
    return lambda i: _bf(where[i][0][where[i][1:]])


def _attn_fill(n_mem, n_loop, n_pre):
    n = 2 * (n_loop + n_pre)

    def head_token(axis):
        i = jax.lax.broadcasted_iota(jnp.int32, (n, n), axis)
        in_loop = i < 2 * n_loop
        second = jnp.where(i >= jnp.where(in_loop, n_loop, 2 * n_loop + n_pre), 1, 0)
        return second, jnp.where(in_loop, i - second * n_loop, i - n_loop - second * n_pre)

    (hq, tq), (hk, tk) = head_token(0), head_token(1)
    causal = jnp.where((tq < n_mem) | (tq >= tk), 0.0, -1e9 * LOG2E)
    return jnp.where(hq == hk, causal, -np.inf).astype(F32)


def _kernel(x_hbm, mem0_hbm, wq_hbm, wk_hbm, wv_hbm, wo_hbm, w1_hbm, w2_hbm, w3_hbm,
            w4_hbm, c_hbm, wmod_hbm, out_hbm,
            x1buf, hbuf, hn_v, mod_v, w1_v, w1_x, w2_v, w3_v, w4_v, sems,
            *, S, D, H, DH, M, SEG, FF):
    NSEG = S // SEG
    NX = NL - M
    NP = SEG - NX
    HP = H // 2
    NCT = D // LANES
    DK = D // 2
    scale = float(DH) ** -0.5 * LOG2E

    def mod(i):
        return mod_v[0:1, i * D:(i + 1) * D]

    cp_b = [pltpu.make_async_copy(s_.bitcast(U32), d_, sems.at[i])
            for i, (s_, d_) in enumerate(
                ((w1_hbm, w1_v), (w2_hbm, w2_v), (w3_hbm, w3_v), (w4_hbm, w4_v)))]

    def attention(x_v, xpre, wqkv, wo_v, pre, hnext, aprev, wmod_v, hpre,
                  c_v, mem0_v, fill_v, wsem, msem):
        x32 = x_hbm.bitcast(U32)
        wmod32 = wmod_hbm.bitcast(U32)
        cp_xpre = pltpu.make_async_copy(x32.at[:, pl.ds(NX // 2, NP // 2), :], xpre, sems.at[4])
        cp_x = pltpu.make_async_copy(x32, x_v, sems.at[5])
        cp_o = pltpu.make_async_copy(wo_hbm.bitcast(U32), wo_v, sems.at[6])
        mcols = [(i * DK, DK) for i in range(4)] + [(2 * D, 3 * D), (5 * D, D)]
        cp_m = [pltpu.make_async_copy(wmod32.at[:, pl.ds(a, n)], wmod_v.at[:, pl.ds(a, n)],
                                      msem.at[i]) for i, (a, n) in enumerate(mcols)]

        def fetch_pair(hp):
            for mat, w in enumerate((wq_hbm, wk_hbm, wv_hbm)):
                for par in range(2):
                    pltpu.make_async_copy(w.bitcast(U32).at[:, par, hp, :],
                                          wqkv.at[6 * hp + 2 * mat + par], wsem.at[hp]).start()

        cp_c = pltpu.make_async_copy(c_hbm, c_v, sems.at[7])
        cp_mem = pltpu.make_async_copy(mem0_hbm, mem0_v, sems.at[8])
        for cp in [cp_c, cp_mem, cp_xpre] + cp_m[:4]:
            cp.start()
        fetch_pair(0)
        first_pairs = 10

        fill_v[...] = _attn_fill(M, NL, NP)
        cp_c.wait()
        cp_mem.wait()
        cv = c_v[...].astype(F32)
        silu_c = jnp.broadcast_to(cv * jax.nn.sigmoid(cv), (16, D)).astype(BF16)

        def modulation(i):
            a, n = mcols[i]
            cp_m[i].wait()
            mod_v[:, a:a + n] = _dot(silu_c, _bf(wmod_v[:, a:a + n]))[0:8]

        cp_xpre.wait()
        x1buf[0:NSEG * NP, :] = _ln(_bf(xpre[...]).astype(F32).reshape(NSEG * NP, D))
        for i in range(4):
            modulation(i)
        for hp in range(1, first_pairs):
            fetch_pair(hp)
        sa = mod(0)
        ca1 = 1.0 + mod(1)
        RH = NSEG * NP // 2
        for r in range(0, RH, 16):
            _st_store_lhs(hpre, r // 2, x1buf[r:r + 16, :] * ca1 + sa,
                          x1buf[RH + r:RH + r + 16, :] * ca1 + sa)

        def pre_body(hp, _):
            @pl.when(hp == 3)
            def _():
                for later in range(first_pairs, HP):
                    fetch_pair(later)
                for cp in [cp_x, cp_o] + cp_m[4:] + cp_b:
                    cp.start()

            slabs = wqkv.at[pl.ds(6 * hp, 6)]
            pltpu.make_async_copy(slabs, slabs, wsem.at[hp]).wait()
            for mat in range(3):
                even = wqkv[6 * hp + 2 * mat]
                odd = wqkv[6 * hp + 2 * mat + 1]
                w0 = (even & 0xFFFF) | (odd << 16)
                w1 = (even >> 16) | (odd & np.uint32(0xFFFF0000))
                wqkv[6 * hp + 2 * mat] = w0
                wqkv[6 * hp + 2 * mat + 1] = w1
                b11, b21, b12, b22 = (_bf(w[i * DK // 2:(i + 1) * DK // 2])
                                      for w in (w0, w1) for i in range(2))
                q1, q3, q4, q6, q7 = (v.astype(BF16) for v in _st_rhs(b11, b12, b21, b22))
                rhs = (q1, b11, q3, q4, b22, q6, q7)
                cs = _st_matmul(lambda i: _bf(hpre[i]), lambda i: rhs[i])
                for t in range(2):
                    ab = [v.reshape(NSEG // 2, NP, DH) for v in cs[2 * t:2 * t + 2]]
                    pre[3 * hp + mat, t * RH:(t + 1) * RH, :] = _words(
                        jnp.concatenate(ab, axis=1).reshape(2 * RH, DH))
            return 0

        with jax.named_scope("P_pre"):
            jax.lax.fori_loop(0, HP, pre_body, 0)

        def modulated(s):
            return _ln(_bf(x_v[s]).astype(F32)[0:NX]) * ca1 + sa

        def retire(i):
            for r0 in range(0, SEG, 16):
                hn = []
                for u in range(2):
                    r = _rows((2 * i + u) * SEG + r0, 16)
                    x = _bf(x_v[2 * i + u, r0 // 2:r0 // 2 + 8, :]).astype(F32)
                    x1 = x + mod(2) * aprev[u, r0:r0 + 16, :]
                    h = _ln(x1) * (1.0 + mod(4)) + mod(3)
                    x1buf[r, :] = x1
                    hbuf[r, :] = h
                    hn.append(_ln(h))
                _st_store_lhs(hn_v, i * (SEG // 2) + r0 // 2, *hn)

        cp_x.wait()
        cp_o.wait()
        modulation(4)
        hnext[...] = modulated(0)
        aprev[...] = jnp.zeros(aprev.shape, F32)

        def seg_step(s, u, mem, held):
            lhs = jnp.concatenate([mem, hnext[...]], axis=0).astype(BF16)
            hnext[...] = modulated(jnp.minimum(s + 1, NSEG - 1))
            rp = _rows(s * NP, NP)
            fill = fill_v[...]
            vis = fill == 0.0
            outs = []

            def join(mat, hp, a, b):
                ab = jnp.concatenate([a, b], axis=0).astype(BF16)
                return jnp.concatenate([ab, _bf(pre[3 * hp + mat, rp, :])], axis=0)

            def proj(mat, hp):
                j = 6 * hp + 2 * mat
                return join(mat, hp, _dot(lhs, _bf(wqkv[j])), _dot(lhs, _bf(wqkv[j + 1])))

            def probs(q, k):
                sc = jnp.where(vis, _dot_nt(q, k) * scale, fill)
                e = jnp.exp2(sc - jnp.max(sc, axis=-1, keepdims=True))
                den = jnp.sum(e, axis=-1, keepdims=True)
                inv = pl.reciprocal(den, approx=True)
                inv = inv * (2.0 - den * inv)
                return (e * inv).astype(BF16)

            def finish(hp, p, v):
                o = _dot(p, v)
                for t in range(2):
                    rows = [o[t * NL:(t + 1) * NL]]
                    late = o[2 * NL + t * NP:2 * NL + (t + 1) * NP]
                    if u == 0:
                        held.append(late)
                    else:
                        rows += [held[2 * hp + t], late]
                    outs.append(_words(jnp.concatenate(rows, axis=0)))

            def wo_part(h0, h1, j):
                return _dot(_bf(jnp.concatenate(outs[h0:h1], axis=1)),
                            _bf(wo_v[h0 * DH // 2:h1 * DH // 2, j * LANES:(j + 1) * LANES]))

            q, k, v, pr = {}, {}, {}, {}
            js = [2, 3, 0, 1]
            lo = [_dot(lhs[:, :DK], _bf(wqkv[j, 0:DK // 2, :])) for j in js]
            full = [_dot(lhs[:, DK:], _bf(wqkv[j, DK // 2:DK, :])) + a for a, j in zip(lo, js)]
            k[0] = join(1, 0, full[0], full[1])
            q[0] = join(0, 0, full[2], full[3])
            for hp in range(1, HP):
                k[hp] = proj(1, hp)
                pr[hp - 1] = probs(q[hp - 1], k[hp - 1])
                q[hp] = proj(0, hp)
                if hp >= 2:
                    finish(hp - 2, pr[hp - 2], v[hp - 2])
                v[hp - 1] = proj(2, hp - 1)
            v[HP - 1] = proj(2, HP - 1)
            pr[HP - 1] = probs(q[HP - 1], k[HP - 1])
            acc = [wo_part(0, HP, 0)]
            finish(HP - 2, pr[HP - 2], v[HP - 2])
            acc += [wo_part(0, HP, j) for j in range(1, NCT // 2)]
            finish(HP - 1, pr[HP - 1], v[HP - 1])
            acc += [wo_part(0, HP, j) for j in range(NCT // 2, NCT)]
            res = jnp.concatenate([wo_part(HP, H, j) + acc[j] for j in range(NCT)], axis=1)
            aprev[u, 0:NX, :] = res[M:NL]
            if u == 1:
                aprev[0, NX:SEG, :] = res[NL:NL + NP]
                aprev[1, NX:SEG, :] = res[NL + NP:]
            return res[:M]

        def seg_body(i, mem):
            retire(jnp.maximum(i - 1, 0))
            held = []
            for u in range(2):
                mem = seg_step(2 * i + u, u, mem, held)
            return mem

        with jax.named_scope("P_seg"):
            jax.lax.fori_loop(0, NSEG // 2, seg_body, mem0_v[...].astype(F32))
        for cp in cp_b:
            cp.wait()
        modulation(5)
        retire(NSEG // 2 - 1)
        _st_prepare(w1_v, w1_x, 0, 1)

    pl.run_scoped(
        attention,
        pltpu.VMEM((NSEG, SEG // 2, D), U32),
        pltpu.VMEM((NSEG, NP // 2, D), U32),
        pltpu.VMEM((3 * H, D // 2, DH), U32),
        pltpu.VMEM((H * DH // 2, D), U32),
        pltpu.VMEM((3 * HP, NSEG * NP, DH), U32),
        pltpu.VMEM((NX, D), F32),
        pltpu.VMEM((2, SEG, D), F32),
        pltpu.VMEM((D // 2, 6 * D), U32),
        pltpu.VMEM((7, NSEG * NP // 4, DK), U32),
        pltpu.VMEM((1, D), BF16),
        pltpu.VMEM((M, D), BF16),
        pltpu.VMEM((2 * (NL + NP),) * 2, F32),
        pltpu.SemaphoreType.DMA((HP,)),
        pltpu.SemaphoreType.DMA((6,)))

    def mixer(ubuf, w2_x, w3_x, w4_x, ynext, obuf, osem):
        ubuf[:, 0:PAD, :] = jnp.zeros((NCT, PAD, LANES), F32)
        ubuf[:, PAD + S:2 * PAD + S, :] = jnp.zeros((NCT, PAD, LANES), F32)

        def stage1(c, _):
            _st_prepare(w2_v, w2_x, c, S // TC)
            _st_prepare(w3_v, w3_x, c, S // TC)
            r = _rows(c * (TC // 4), TC // 4)
            for j in range(NCT // 2):
                cs = _st_matmul(lambda i: _bf(hn_v[i, r, :]),
                                _st_weights(w1_v, w1_x, 0, DK, j * LANES, LANES))
                for i, v in enumerate(cs):
                    u = _gelu(v)
                    for g in range(TC // (2 * SEG)):
                        ubuf[(i % 2) * (NCT // 2) + j,
                             _rows(c * TC + (2 * g + i // 2) * SEG + PAD, SEG), :] = (
                                 u[g * SEG:(g + 1) * SEG])
            return 0

        with jax.named_scope("P_s1"):
            jax.lax.fori_loop(0, S // TC, stage1, 0)

        def stage2(c, _):
            _st_prepare(w4_v, w4_x, c, S // TC)
            th = TC // 2
            shifts = (-1, 1, -2, 2)
            top, bottom = (jnp.concatenate(
                [ubuf[j, pl.ds(c * TC + t * th + PAD + shifts[j * 4 // NCT], th), :]
                 for j in range(NCT)], axis=1) for t in range(2))
            lhs = _st_lhs(top[:, :DK], top[:, DK:], bottom[:, :DK], bottom[:, DK:])
            for j in range(0, DK, LANES):
                cs = _st_matmul(lambda i: lhs[i], _st_weights(w2_v, w2_x, 0, DK, j, LANES))
                for i, v in enumerate(cs):
                    r = _rows(c * TC + (i // 2) * th, th)
                    cc = slice((i % 2) * DK + j, (i % 2) * DK + j + LANES)
                    hbuf[r, cc] = hbuf[r, cc] + v
            return 0

        with jax.named_scope("P_s2"):
            jax.lax.fori_loop(0, S // TC, stage2, 0)

        def ffn_input(c, r):
            _st_store_lhs(ynext.at[c % 2], r // 2, _ln(hbuf[_rows(c * TB + r, 16), :]),
                          _ln(hbuf[_rows(c * TB + TB // 2 + r, 16), :]))

        def out_copy(c):
            return pltpu.make_async_copy(obuf.at[c], out_hbm.at[c], osem.at[c])

        def stage3(c, _):
            nf = FF // 2 // LANES
            pieces = list(range(0, TB // 2, 16))
            due = {(i + 1) * (nf - 1) // len(pieces): r for i, r in enumerate(pieces)}

            def up(j):
                if j in due:
                    ffn_input(jnp.where(c + 1 < S // TB, c + 1, 0), due[j])
                cs = _st_matmul(lambda i: _bf(ynext[c % 2, i]),
                                _st_weights(w3_v, w3_x, 0, DK, j * LANES, LANES))
                return [_words(t) for t in _st_lhs(*(_gelu(v) for v in cs))]

            edges = [0] + list(range(nf % FG or FG, nf + 1, FG))
            groups = list(zip(edges[:-1], edges[1:]))
            ups = {j: up(j) for j in range(*groups[0])}
            ms = {}
            for g, (j0, j1) in enumerate(groups):
                if g + 1 < len(groups):
                    ups.update({j: up(j) for j in range(*groups[g + 1])})
                ts = [_bf(jnp.concatenate([ups[j][i] for j in range(j0, j1)], axis=1))
                      for i in range(7)]
                for n in range(0, DK, LANES):
                    w = _st_weights(w4_v, w4_x, j0 * LANES, (j1 - j0) * LANES, n, LANES)
                    for i in range(7):
                        d = _dot(ts[i], w(i))
                        ms[n, i] = d + ms[n, i] if g else d
            for n in range(0, DK, LANES):
                for i, z in enumerate(_st_out(*(ms[n, i] for i in range(7)))):
                    r0 = (i // 2) * (TB // 2)
                    r = _rows(c * TB + r0, TB // 2)
                    cc = slice((i % 2) * DK + n, (i % 2) * DK + n + LANES)
                    obuf[c, r0:r0 + TB // 2, cc] = (
                        x1buf[r, cc] + mod(5)[:, cc] * (hbuf[r, cc] + z)).astype(obuf.dtype)
            out_copy(c).start()
            return 0

        for r in range(0, TB // 2, 16):
            ffn_input(0, r)
        with jax.named_scope("P_s3"):
            jax.lax.fori_loop(0, S // TB, stage3, 0)
        for c in range(S // TB):
            out_copy(c).wait()

    pl.run_scoped(
        mixer,
        pltpu.VMEM((NCT, S + 2 * PAD, LANES), F32),
        pltpu.VMEM((3, D // 4, DK), U32),
        pltpu.VMEM((3, D // 4, FF // 2), U32),
        pltpu.VMEM((3, FF // 4, DK), U32),
        pltpu.VMEM((2, 7, TB // 4, DK), U32),
        pltpu.VMEM(out_hbm.shape, out_hbm.dtype),
        pltpu.SemaphoreType.DMA((S // TB,)))


@functools.partial(jax.jit, static_argnames=("A_seg_len",))
def pallas_adaLN_cond__memory_aug_recurrent_mem_tr__mixer_s_mlp__prompt_kernel(
    A_x, A_mem0, A_Wq, A_Wk, A_Wv, A_Wo, A_seg_len, B_x, B_w1, B_w2, B_w3, B_w4, c, w_mod,
):
    del B_x
    B, S, D = A_x.shape
    _, H, DH = A_Wq.shape
    M = A_mem0.shape[1]
    SEG = int(A_seg_len)
    FF = B_w3.shape[1]
    assert B == 1 and DH == LANES and M == 8 and SEG == 32 and S % SEG == 0
    NSEG = S // SEG

    hbm = pl.BlockSpec(memory_space=pl.ANY)
    out = pl.pallas_call(
        functools.partial(_kernel, S=S, D=D, H=H, DH=DH, M=M, SEG=SEG, FF=FF),
        out_shape=jax.ShapeDtypeStruct((S // TB, TB, D), A_x.dtype),
        in_specs=[hbm] * 12,
        out_specs=hbm,
        scratch_shapes=[
            pltpu.VMEM((S, D), F32),
            pltpu.VMEM((S, D), F32),
            pltpu.VMEM((7, S // 4, D // 2), U32),
            pltpu.VMEM((8, 6 * D), F32),
            pltpu.VMEM((D // 2, D), U32),
            pltpu.VMEM((3, D // 4, D // 2), U32),
            pltpu.VMEM((D // 2, D), U32),
            pltpu.VMEM((D // 2, FF), U32),
            pltpu.VMEM((FF // 2, D), U32),
            pltpu.SemaphoreType.DMA((9,)),
        ],
        compiler_params=pltpu.CompilerParams(vmem_limit_bytes=124 * 2**20),
        name="adaln_rmt_mixer",
    )(
        A_x.reshape(NSEG, SEG, D), A_mem0.reshape(M, D),
        A_Wq.reshape(D // 2, 2, H, DH), A_Wk.reshape(D // 2, 2, H, DH),
        A_Wv.reshape(D // 2, 2, H, DH),
        A_Wo.reshape(H * DH, D), B_w1, B_w2, B_w3, B_w4, c, w_mod,
    )
    return out.reshape(B, S, D)
```

```python
import functools

import jax
import jax.numpy as jnp
import numpy as np
import jax.experimental.pallas as pl
import jax.experimental.pallas.tpu as pltpu

F32 = jnp.float32
BF16 = jnp.bfloat16
U32 = jnp.uint32
LANES = 128
EPS = 1e-5
LOG2E = 1.4426950408889634
NL = 32
PAD = 8
TC = 256
TB = 128
FG = 4


def _ln(x):
    m = jnp.mean(x, axis=-1, keepdims=True)
    d = x - m
    v = jnp.mean(d * d, axis=-1, keepdims=True)
    return d * jax.lax.rsqrt(v + EPS)


def _gelu(x):
    c0 = float(np.sqrt(2.0 / np.pi))
    inner = x * (c0 + (c0 * 0.044715) * (x * x))
    hx = 0.5 * x
    return hx + hx * jnp.tanh(inner)


def _dot(a, b):
    return jnp.dot(a, b, preferred_element_type=F32)


def _dot_nt(a, b):
    return jax.lax.dot_general(a, b, (((1,), (1,)), ((), ())),
                               preferred_element_type=F32)


def _bf(words):
    return pltpu.bitcast(words, BF16)


def _words(x):
    return pltpu.bitcast(x.astype(BF16), U32)


def _rows(start, n):
    return pl.ds(pl.multiple_of(start, 8), n)


def _st_lhs(a11, a12, a21, a22):
    return [v.astype(BF16) for v in
            (a11 + a22, a21 + a22, a11, a22, a11 + a12, a21 - a11, a12 - a22)]


def _st_rhs(b11, b12, b21, b22):
    b11, b12, b21, b22 = (b.astype(F32) for b in (b11, b12, b21, b22))
    return b11 + b22, b12 - b22, b21 - b11, b11 + b12, b21 + b22


def _st_out(m1, m2, m3, m4, m5, m6, m7):
    return (m1 + m4) + (m7 - m5), m3 + m5, m2 + m4, (m1 - m2) + (m3 + m6)


def _st_matmul(lhs, rhs):
    m2 = _dot(lhs(1), rhs(1))
    m4 = _dot(lhs(3), rhs(3))
    m1 = _dot(lhs(0), rhs(0))
    c21, c11, c22 = m2 + m4, m1 + m4, m1 - m2
    c11 = _dot(lhs(6), rhs(6)) + c11
    m5 = _dot(lhs(4), rhs(4))
    m3 = _dot(lhs(2), rhs(2))
    return c11 - m5, m3 + m5, c21, _dot(lhs(5), rhs(5)) + (c22 + m3)


def _st_store_lhs(dst, word_row, top, bottom):
    n, k = top.shape[0] // 2, top.shape[1] // 2
    for i, v in enumerate(_st_lhs(top[:, :k], top[:, k:], bottom[:, :k], bottom[:, k:])):
        dst[i, _rows(word_row, n), :] = _words(v)


def _st_prepare(w_v, extra, part, parts):
    kr, kc = w_v.shape[0] // 2, w_v.shape[1] // 2
    rows = kr // parts
    for r in range(0, rows, 8):
        r1, r2 = _rows(part * rows + r, 8), _rows(kr + part * rows + r, 8)
        for j in range(0, kc, 2 * LANES):
            c1, c2 = slice(j, j + 2 * LANES), slice(kc + j, kc + j + 2 * LANES)
            q1, q3, q4, q6, q7 = (_words(v) for v in _st_rhs(
                *(_bf(w_v[r_, c_]) for r_ in (r1, r2) for c_ in (c1, c2))))
            w_v[r1, c2] = q3
            w_v[r2, c1] = q4
            extra[0, r1, c1] = q1
            extra[1, r1, c1] = q6
            extra[2, r1, c1] = q7


def _st_weights(w_v, extra, k0, nk, c0, nc):
    kr, kc = w_v.shape[0] // 2, w_v.shape[1] // 2
    ra, rb = slice(k0 // 2, (k0 + nk) // 2), slice(kr + k0 // 2, kr + (k0 + nk) // 2)
    ca, cb = slice(c0, c0 + nc), slice(kc + c0, kc + c0 + nc)
    where = ((extra, 0, ra, ca), (w_v, ra, ca), (w_v, ra, cb), (w_v, rb, ca),
             (w_v, rb, cb), (extra, 1, ra, ca), (extra, 2, ra, ca))
    return lambda i: _bf(where[i][0][where[i][1:]])


def _attn_fill(n_mem, n_loop, n_pre):
    n = 2 * (n_loop + n_pre)

    def head_token(axis):
        i = jax.lax.broadcasted_iota(jnp.int32, (n, n), axis)
        in_loop = i < 2 * n_loop
        second = jnp.where(i >= jnp.where(in_loop, n_loop, 2 * n_loop + n_pre), 1, 0)
        return second, jnp.where(in_loop, i - second * n_loop, i - n_loop - second * n_pre)

    (hq, tq), (hk, tk) = head_token(0), head_token(1)
    causal = jnp.where((tq < n_mem) | (tq >= tk), 0.0, -1e9 * LOG2E)
    return jnp.where(hq == hk, causal, -np.inf).astype(F32)


def _kernel(x_hbm, mem0_hbm, wq_hbm, wk_hbm, wv_hbm, wo_hbm, w1_hbm, w2_hbm, w3_hbm,
            w4_hbm, c_hbm, wmod_hbm, out_hbm,
            x1buf, hbuf, hn_v, mod_v, w1_v, w1_x, w2_v, w3_v, w4_v, sems,
            *, S, D, H, DH, M, SEG, FF):
    NSEG = S // SEG
    NX = NL - M
    NP = SEG - NX
    HP = H // 2
    NCT = D // LANES
    DK = D // 2
    scale = float(DH) ** -0.5 * LOG2E

    def mod(i):
        return mod_v[0:1, i * D:(i + 1) * D]

    cp_b = [pltpu.make_async_copy(s_.bitcast(U32), d_, sems.at[i])
            for i, (s_, d_) in enumerate(
                ((w1_hbm, w1_v), (w2_hbm, w2_v), (w3_hbm, w3_v), (w4_hbm, w4_v)))]

    def attention(x_v, xpre, wqkv, wo_v, pre, hnext, aprev, wmod_v, hpre,
                  c_v, mem0_v, fill_v, wsem, msem):
        x32 = x_hbm.bitcast(U32)
        wmod32 = wmod_hbm.bitcast(U32)
        cp_xpre = pltpu.make_async_copy(x32.at[:, pl.ds(NX // 2, NP // 2), :], xpre, sems.at[4])
        cp_x = pltpu.make_async_copy(x32, x_v, sems.at[5])
        cp_o = pltpu.make_async_copy(wo_hbm.bitcast(U32), wo_v, sems.at[6])
        mcols = [(i * DK, DK) for i in range(4)] + [(2 * D, 3 * D), (5 * D, D)]
        cp_m = [pltpu.make_async_copy(wmod32.at[:, pl.ds(a, n)], wmod_v.at[:, pl.ds(a, n)],
                                      msem.at[i]) for i, (a, n) in enumerate(mcols)]

        def fetch_pair(hp):
            for mat, w in enumerate((wq_hbm, wk_hbm, wv_hbm)):
                for par in range(2):
                    pltpu.make_async_copy(w.bitcast(U32).at[:, par, hp, :],
                                          wqkv.at[6 * hp + 2 * mat + par], wsem.at[hp]).start()

        cp_c = pltpu.make_async_copy(c_hbm, c_v, sems.at[7])
        cp_mem = pltpu.make_async_copy(mem0_hbm, mem0_v, sems.at[8])
        for cp in [cp_c, cp_mem, cp_xpre] + cp_m[:4]:
            cp.start()
        fetch_pair(0)
        first_pairs = 10

        fill_v[...] = _attn_fill(M, NL, NP)
        cp_c.wait()
        cp_mem.wait()
        cv = c_v[...].astype(F32)
        silu_c = jnp.broadcast_to(cv * jax.nn.sigmoid(cv), (16, D)).astype(BF16)

        def modulation(i):
            a, n = mcols[i]
            cp_m[i].wait()
            mod_v[:, a:a + n] = _dot(silu_c, _bf(wmod_v[:, a:a + n]))[0:8]

        cp_xpre.wait()
        x1buf[0:NSEG * NP, :] = _ln(_bf(xpre[...]).astype(F32).reshape(NSEG * NP, D))
        for i in range(4):
            modulation(i)
        for hp in range(1, first_pairs):
            fetch_pair(hp)
        sa = mod(0)
        ca1 = 1.0 + mod(1)
        RH = NSEG * NP // 2
        for r in range(0, RH, 16):
            _st_store_lhs(hpre, r // 2, x1buf[r:r + 16, :] * ca1 + sa,
                          x1buf[RH + r:RH + r + 16, :] * ca1 + sa)

        def pre_body(hp, _):
            @pl.when(hp == 3)
            def _():
                for later in range(first_pairs, HP):
                    fetch_pair(later)
                for cp in [cp_x, cp_o] + cp_m[4:] + cp_b:
                    cp.start()

            slabs = wqkv.at[pl.ds(6 * hp, 6)]
            pltpu.make_async_copy(slabs, slabs, wsem.at[hp]).wait()
            for mat in range(3):
                even = wqkv[6 * hp + 2 * mat]
                odd = wqkv[6 * hp + 2 * mat + 1]
                w0 = (even & 0xFFFF) | (odd << 16)
                w1 = (even >> 16) | (odd & np.uint32(0xFFFF0000))
                wqkv[6 * hp + 2 * mat] = w0
                wqkv[6 * hp + 2 * mat + 1] = w1
                b11, b21, b12, b22 = (_bf(w[i * DK // 2:(i + 1) * DK // 2])
                                      for w in (w0, w1) for i in range(2))
                q1, q3, q4, q6, q7 = (v.astype(BF16) for v in _st_rhs(b11, b12, b21, b22))
                rhs = (q1, b11, q3, q4, b22, q6, q7)
                cs = _st_matmul(lambda i: _bf(hpre[i]), lambda i: rhs[i])
                for t in range(2):
                    ab = [v.reshape(NSEG // 2, NP, DH) for v in cs[2 * t:2 * t + 2]]
                    pre[3 * hp + mat, t * RH:(t + 1) * RH, :] = _words(
                        jnp.concatenate(ab, axis=1).reshape(2 * RH, DH))
            return 0

        jax.lax.fori_loop(0, HP, pre_body, 0)

        def modulated(s):
            return _ln(_bf(x_v[s]).astype(F32)[0:NX]) * ca1 + sa

        def retire(i):
            for r0 in range(0, SEG, 16):
                hn = []
                for u in range(2):
                    r = _rows((2 * i + u) * SEG + r0, 16)
                    x = _bf(x_v[2 * i + u, r0 // 2:r0 // 2 + 8, :]).astype(F32)
                    x1 = x + mod(2) * aprev[u, r0:r0 + 16, :]
                    h = _ln(x1) * (1.0 + mod(4)) + mod(3)
                    x1buf[r, :] = x1
                    hbuf[r, :] = h
                    hn.append(_ln(h))
                _st_store_lhs(hn_v, i * (SEG // 2) + r0 // 2, *hn)

        cp_x.wait()
        cp_o.wait()
        modulation(4)
        hnext[...] = modulated(0)
        aprev[...] = jnp.zeros(aprev.shape, F32)

        def seg_step(s, u, mem, held):
            lhs = jnp.concatenate([mem, hnext[...]], axis=0).astype(BF16)
            hnext[...] = modulated(jnp.minimum(s + 1, NSEG - 1))
            rp = _rows(s * NP, NP)
            fill = fill_v[...]
            vis = fill == 0.0
            outs = []

            def join(mat, hp, a, b):
                ab = jnp.concatenate([a, b], axis=0).astype(BF16)
                return jnp.concatenate([ab, _bf(pre[3 * hp + mat, rp, :])], axis=0)

            def proj(mat, hp):
                j = 6 * hp + 2 * mat
                return join(mat, hp, _dot(lhs, _bf(wqkv[j])), _dot(lhs, _bf(wqkv[j + 1])))

            def probs(q, k):
                sc = jnp.where(vis, _dot_nt(q, k) * scale, fill)
                e = jnp.exp2(sc - jnp.max(sc, axis=-1, keepdims=True))
                den = jnp.sum(e, axis=-1, keepdims=True)
                inv = pl.reciprocal(den, approx=True)
                inv = inv * (2.0 - den * inv)
                return (e * inv).astype(BF16)

            def finish(hp, p, v):
                o = _dot(p, v)
                for t in range(2):
                    rows = [o[t * NL:(t + 1) * NL]]
                    late = o[2 * NL + t * NP:2 * NL + (t + 1) * NP]
                    if u == 0:
                        held.append(late)
                    else:
                        rows += [held[2 * hp + t], late]
                    outs.append(_words(jnp.concatenate(rows, axis=0)))

            def wo_part(h0, h1, j):
                return _dot(_bf(jnp.concatenate(outs[h0:h1], axis=1)),
                            _bf(wo_v[h0 * DH // 2:h1 * DH // 2, j * LANES:(j + 1) * LANES]))

            q, k, v, pr = {}, {}, {}, {}
            js = [2, 3, 0, 1]
            lo = [_dot(lhs[:, :DK], _bf(wqkv[j, 0:DK // 2, :])) for j in js]
            full = [_dot(lhs[:, DK:], _bf(wqkv[j, DK // 2:DK, :])) + a for a, j in zip(lo, js)]
            k[0] = join(1, 0, full[0], full[1])
            q[0] = join(0, 0, full[2], full[3])
            for hp in range(1, HP):
                k[hp] = proj(1, hp)
                pr[hp - 1] = probs(q[hp - 1], k[hp - 1])
                q[hp] = proj(0, hp)
                if hp >= 2:
                    finish(hp - 2, pr[hp - 2], v[hp - 2])
                v[hp - 1] = proj(2, hp - 1)
            v[HP - 1] = proj(2, HP - 1)
            pr[HP - 1] = probs(q[HP - 1], k[HP - 1])
            acc = [wo_part(0, HP, 0)]
            finish(HP - 2, pr[HP - 2], v[HP - 2])
            acc += [wo_part(0, HP, j) for j in range(1, NCT // 2)]
            finish(HP - 1, pr[HP - 1], v[HP - 1])
            acc += [wo_part(0, HP, j) for j in range(NCT // 2, NCT)]
            res = jnp.concatenate([wo_part(HP, H, j) + acc[j] for j in range(NCT)], axis=1)
            aprev[u, 0:NX, :] = res[M:NL]
            if u == 1:
                aprev[0, NX:SEG, :] = res[NL:NL + NP]
                aprev[1, NX:SEG, :] = res[NL + NP:]
            return res[:M]

        def seg_body(i, mem):
            retire(jnp.maximum(i - 1, 0))
            held = []
            for u in range(2):
                mem = seg_step(2 * i + u, u, mem, held)
            return mem

        jax.lax.fori_loop(0, NSEG // 2, seg_body, mem0_v[...].astype(F32))
        for cp in cp_b:
            cp.wait()
        modulation(5)
        retire(NSEG // 2 - 1)
        _st_prepare(w1_v, w1_x, 0, 1)

    pl.run_scoped(
        attention,
        pltpu.VMEM((NSEG, SEG // 2, D), U32),
        pltpu.VMEM((NSEG, NP // 2, D), U32),
        pltpu.VMEM((3 * H, D // 2, DH), U32),
        pltpu.VMEM((H * DH // 2, D), U32),
        pltpu.VMEM((3 * HP, NSEG * NP, DH), U32),
        pltpu.VMEM((NX, D), F32),
        pltpu.VMEM((2, SEG, D), F32),
        pltpu.VMEM((D // 2, 6 * D), U32),
        pltpu.VMEM((7, NSEG * NP // 4, DK), U32),
        pltpu.VMEM((1, D), BF16),
        pltpu.VMEM((M, D), BF16),
        pltpu.VMEM((2 * (NL + NP),) * 2, F32),
        pltpu.SemaphoreType.DMA((HP,)),
        pltpu.SemaphoreType.DMA((6,)))

    def mixer(ubuf, w2_x, w3_x, w4_x, ynext, obuf, osem):
        ubuf[:, 0:PAD, :] = jnp.zeros((NCT, PAD, LANES), F32)
        ubuf[:, PAD + S:2 * PAD + S, :] = jnp.zeros((NCT, PAD, LANES), F32)

        def stage1(c, _):
            _st_prepare(w2_v, w2_x, c, S // TC)
            _st_prepare(w3_v, w3_x, c, S // TC)
            r = _rows(c * (TC // 4), TC // 4)
            for j in range(NCT // 2):
                cs = _st_matmul(lambda i: _bf(hn_v[i, r, :]),
                                _st_weights(w1_v, w1_x, 0, DK, j * LANES, LANES))
                for i, v in enumerate(cs):
                    u = _gelu(v)
                    for g in range(TC // (2 * SEG)):
                        ubuf[(i % 2) * (NCT // 2) + j,
                             _rows(c * TC + (2 * g + i // 2) * SEG + PAD, SEG), :] = (
                                 u[g * SEG:(g + 1) * SEG])
            return 0

        jax.lax.fori_loop(0, S // TC, stage1, 0)

        def stage2(c, _):
            _st_prepare(w4_v, w4_x, c, S // TC)
            th = TC // 2
            shifts = (-1, 1, -2, 2)
            top, bottom = (jnp.concatenate(
                [ubuf[j, pl.ds(c * TC + t * th + PAD + shifts[j * 4 // NCT], th), :]
                 for j in range(NCT)], axis=1) for t in range(2))
            lhs = _st_lhs(top[:, :DK], top[:, DK:], bottom[:, :DK], bottom[:, DK:])
            for j in range(0, DK, LANES):
                cs = _st_matmul(lambda i: lhs[i], _st_weights(w2_v, w2_x, 0, DK, j, LANES))
                for i, v in enumerate(cs):
                    r = _rows(c * TC + (i // 2) * th, th)
                    cc = slice((i % 2) * DK + j, (i % 2) * DK + j + LANES)
                    hbuf[r, cc] = hbuf[r, cc] + v
            return 0

        jax.lax.fori_loop(0, S // TC, stage2, 0)

        def ffn_input(c, r):
            _st_store_lhs(ynext.at[c % 2], r // 2, _ln(hbuf[_rows(c * TB + r, 16), :]),
                          _ln(hbuf[_rows(c * TB + TB // 2 + r, 16), :]))

        def out_copy(c):
            return pltpu.make_async_copy(obuf.at[c], out_hbm.at[c], osem.at[c])

        def stage3(c, _):
            nf = FF // 2 // LANES
            pieces = list(range(0, TB // 2, 16))
            due = {(i + 1) * (nf - 1) // len(pieces): r for i, r in enumerate(pieces)}

            def up(j):
                if j in due:
                    ffn_input(jnp.where(c + 1 < S // TB, c + 1, 0), due[j])
                cs = _st_matmul(lambda i: _bf(ynext[c % 2, i]),
                                _st_weights(w3_v, w3_x, 0, DK, j * LANES, LANES))
                return [_words(t) for t in _st_lhs(*(_gelu(v) for v in cs))]

            edges = [0] + list(range(nf % FG or FG, nf + 1, FG))
            groups = list(zip(edges[:-1], edges[1:]))
            ups = {j: up(j) for j in range(*groups[0])}
            ms = {}
            for g, (j0, j1) in enumerate(groups):
                if g + 1 < len(groups):
                    ups.update({j: up(j) for j in range(*groups[g + 1])})
                ts = [_bf(jnp.concatenate([ups[j][i] for j in range(j0, j1)], axis=1))
                      for i in range(7)]
                for n in range(0, DK, LANES):
                    w = _st_weights(w4_v, w4_x, j0 * LANES, (j1 - j0) * LANES, n, LANES)
                    for i in range(7):
                        d = _dot(ts[i], w(i))
                        ms[n, i] = d + ms[n, i] if g else d
            for n in range(0, DK, LANES):
                for i, z in enumerate(_st_out(*(ms[n, i] for i in range(7)))):
                    r0 = (i // 2) * (TB // 2)
                    r = _rows(c * TB + r0, TB // 2)
                    cc = slice((i % 2) * DK + n, (i % 2) * DK + n + LANES)
                    obuf[c, r0:r0 + TB // 2, cc] = (
                        x1buf[r, cc] + mod(5)[:, cc] * (hbuf[r, cc] + z)).astype(obuf.dtype)
            out_copy(c).start()
            return 0

        for r in range(0, TB // 2, 16):
            ffn_input(0, r)
        jax.lax.fori_loop(0, S // TB, stage3, 0)
        for c in range(S // TB):
            out_copy(c).wait()

    pl.run_scoped(
        mixer,
        pltpu.VMEM((NCT, S + 2 * PAD, LANES), F32),
        pltpu.VMEM((3, D // 4, DK), U32),
        pltpu.VMEM((3, D // 4, FF // 2), U32),
        pltpu.VMEM((3, FF // 4, DK), U32),
        pltpu.VMEM((2, 7, TB // 4, DK), U32),
        pltpu.VMEM(out_hbm.shape, out_hbm.dtype),
        pltpu.SemaphoreType.DMA((S // TB,)))


@functools.partial(jax.jit, static_argnames=("A_seg_len",))
def pallas_adaLN_cond__memory_aug_recurrent_mem_tr__mixer_s_mlp__prompt_kernel(
    A_x, A_mem0, A_Wq, A_Wk, A_Wv, A_Wo, A_seg_len, B_x, B_w1, B_w2, B_w3, B_w4, c, w_mod,
):
    del B_x
    B, S, D = A_x.shape
    _, H, DH = A_Wq.shape
    M = A_mem0.shape[1]
    SEG = int(A_seg_len)
    FF = B_w3.shape[1]
    assert B == 1 and DH == LANES and M == 8 and SEG == 32
    assert S % TC == 0 and S % (2 * TB) == 0
    NSEG = S // SEG

    hbm = pl.BlockSpec(memory_space=pl.ANY)
    out = pl.pallas_call(
        functools.partial(_kernel, S=S, D=D, H=H, DH=DH, M=M, SEG=SEG, FF=FF),
        out_shape=jax.ShapeDtypeStruct((S // TB, TB, D), A_x.dtype),
        in_specs=[hbm] * 12,
        out_specs=hbm,
        scratch_shapes=[
            pltpu.VMEM((S, D), F32),
            pltpu.VMEM((S, D), F32),
            pltpu.VMEM((7, S // 4, D // 2), U32),
            pltpu.VMEM((8, 6 * D), F32),
            pltpu.VMEM((D // 2, D), U32),
            pltpu.VMEM((3, D // 4, D // 2), U32),
            pltpu.VMEM((D // 2, D), U32),
            pltpu.VMEM((D // 2, FF), U32),
            pltpu.VMEM((FF // 2, D), U32),
            pltpu.SemaphoreType.DMA((9,)),
        ],
        compiler_params=pltpu.CompilerParams(vmem_limit_bytes=124 * 2**20),
        name="adaln_rmt_mixer",
    )(
        A_x.reshape(NSEG, SEG, D), A_mem0.reshape(M, D),
        A_Wq.reshape(D // 2, 2, H, DH), A_Wk.reshape(D // 2, 2, H, DH),
        A_Wv.reshape(D // 2, 2, H, DH),
        A_Wo.reshape(H * DH, D), B_w1, B_w2, B_w3, B_w4, c, w_mod,
    )
    return out.reshape(B, S, D)
```
